```python
import jax
import jax.numpy as jnp

def _softmax(x, axis=-1):
    return jax.nn.softmax(x, axis=axis)
def _gelu(x):
    return jax.nn.gelu(x, approximate=True)
def _silu(x):
    return jax.nn.silu(x)
def _sigmoid(x):
    return jax.nn.sigmoid(x)
def _layernorm(x, axis=-1, eps=1e-5):
    m = jnp.mean(x, axis=axis, keepdims=True)
    v = jnp.var(x, axis=axis, keepdims=True)
    return (x - m) / jnp.sqrt(v + eps)
def _scatter_add(tgt, idx, src, axis=0):
    return tgt.at[idx].add(src)
def _segment_sum(src, seg, n):
    return jax.ops.segment_sum(src, seg, n)
class _Rng:
    def __init__(self, key):
        self._k = key
    def _next(self):
        self._k, sub = jax.random.split(self._k)
        return sub
    def normal(self, shape):
        return jax.random.normal(self._next(), shape, dtype=jnp.bfloat16)
    def randint(self, lo, hi, shape):
        return jax.random.randint(self._next(), shape, lo, hi, dtype=jnp.int32)
    def uniform(self, shape, lo=0.0, hi=1.0):
        return jax.random.uniform(self._next(), shape, jnp.bfloat16, lo, hi)
    def permutation(self, n):
        return jax.random.permutation(self._next(), n)


kernel_name = 'gated_mix__sliding_block_cached__glu_gated_swiglu__decode'

def setup_inputs():
    _rng = _Rng(jax.random.key(int.from_bytes(__import__("os").urandom(4), "little")))
    _w = (lambda a: (lambda t: t.astype(jnp.bfloat16) if jnp.issubdtype(t.dtype, jnp.floating) else t)(jnp.asarray(a)))
    def _A_setup():
        B, Sq, D = 1, 1, 640
        Hq, Hkv, Sk, Dh = 32, 32, 32768, 192
        assert Hq % Hkv == 0, (Hq, Hkv)
        return {
            "x": _w((lambda *s: _rng.normal(s) * 0.05)(B, Sq, D)),
            "k_cache": _w((lambda *s: _rng.normal(s) * 0.05)(B, Hkv, Sk, Dh)),
            "v_cache": _w((lambda *s: _rng.normal(s) * 0.05)(B, Hkv, Sk, Dh)),
            "wq": _w((lambda *s: _rng.normal(s) * 0.05)(D, Hq * Dh) * (D ** -0.5)),
            "wo": _w((lambda *s: _rng.normal(s) * 0.05)(Hq * Dh, D) * ((Hq * Dh) ** -0.5)),
        }
    _A_in = _A_setup()

    def _B_setup():
        B, S, D, F = 1, 1, 640, 1536
        return {
            "x": _w((lambda *s: _rng.normal(s) * 0.05)(B, S, D)),
            "w1": _w((lambda *s: _rng.normal(s) * 0.05)(D, F) * (2.0 / D) ** 0.5),
            "w3": _w((lambda *s: _rng.normal(s) * 0.05)(D, F) * (2.0 / D) ** 0.5),
            "w2": _w((lambda *s: _rng.normal(s) * 0.05)(F, D) * (2.0 / F) ** 0.5),
        }
    _B_in = _B_setup()

    return {
        "A_x": _A_in["x"],
        "A_k_cache": _A_in["k_cache"],
        "A_v_cache": _A_in["v_cache"],
        "A_wq": _A_in["wq"],
        "A_wo": _A_in["wo"],
        "B_x": _B_in["x"],
        "B_w1": _B_in["w1"],
        "B_w3": _B_in["w3"],
        "B_w2": _B_in["w2"],
        "gate_w": _w((lambda *s: _rng.normal(s) * 0.05)(640)),
    }

def reference(A_x, A_k_cache, A_v_cache, A_wq, A_wo, B_x, B_w1, B_w3, B_w2, gate_w):
    def _A_ref(x, k_cache, v_cache, wq, wo):
        B, Sq, D = x.shape
        Hq, Dh = 32, 192
        Hkv, Sk = k_cache.shape[1], k_cache.shape[2]
        W = min(4096, max(256, Sk // 4))
        rep = Hq // Hkv
        q = (lambda x, *d: x.transpose(*d))((x @ wq).reshape(B, Sq, Hq, Dh), 0, 2, 1, 3)
        k = jnp.repeat(k_cache[:, :, Sk - W:, :], rep, axis=1)
        v = jnp.repeat(v_cache[:, :, Sk - W:, :], rep, axis=1)
        scores = jnp.einsum("bhqd,bhkd->bhqk", q, k) * (Dh ** -0.5)
        p = _softmax(scores, axis=-1)
        o = jnp.einsum("bhqk,bhkd->bhqd", p, v)
        return (lambda x, *d: x.transpose(*d))(o, 0, 2, 1, 3).reshape(B, Sq, Hq * Dh) @ wo

    def _B_ref(x, w1, w3, w2):
        gate = jnp.einsum("bsd,df->bsf", x, w1)
        up = jnp.einsum("bsd,df->bsf", x, w3)
        h = _silu(gate) * up
        out = jnp.einsum("bsf,fd->bsd", h, w2)
        return out

    x = A_x
    g = _sigmoid((x * gate_w).sum(-1, keepdims=True))
    a = _A_ref(x, A_k_cache, A_v_cache, A_wq, A_wo)
    b = _B_ref(x, B_w1, B_w3, B_w2)
    return g * a + (1 - g) * b
```

```python
import functools

import jax
import jax.numpy as jnp
from jax import lax
import jax.experimental.pallas as pl
import jax.experimental.pallas.tpu as pltpu

_LANES = 128
_NBUF = 4
_WO_PIECES = 8


def _kernel(x_hbm, gw_hbm, wq_hbm, k_hbm, v_hbm, wo_hbm, w1_hbm, w3_hbm, w2_hbm,
            o_ref,
            xbuf, gwbuf, wqbuf, wobuf, w1buf, w3buf, w2buf, kbuf, vbuf,
            qbuf, obuf, bbuf,
            sem_small, sem_w, sem_k, sem_v, sem_wo,
            *, H, DH, SK, W, D, F):
    f32 = jnp.float32
    bf16 = jnp.bfloat16
    scale = DH ** -0.5
    s0 = SK - W
    nblk = W // _LANES
    wo_rows = (H * DH) // _WO_PIECES

    def k_copy(h, slot):
        return pltpu.make_async_copy(k_hbm.at[0, h, :, pl.ds(s0, W)], kbuf.at[slot], sem_k.at[slot])

    def v_copy(h, slot):
        return pltpu.make_async_copy(v_hbm.at[0, h, :, pl.ds(s0, W)], vbuf.at[slot], sem_v.at[slot])

    def wo_copy(i):
        return pltpu.make_async_copy(wo_hbm.at[pl.ds(i * wo_rows, wo_rows), :],
                                     wobuf.at[pl.ds(i * wo_rows, wo_rows), :], sem_wo.at[i])

    x_copy = pltpu.make_async_copy(x_hbm, xbuf, sem_small.at[0])
    gw_copy = pltpu.make_async_copy(gw_hbm, gwbuf, sem_small.at[1])
    wq_copy = pltpu.make_async_copy(wq_hbm, wqbuf, sem_w.at[0])
    w1_copy = pltpu.make_async_copy(w1_hbm, w1buf, sem_w.at[1])
    w3_copy = pltpu.make_async_copy(w3_hbm, w3buf, sem_w.at[2])
    w2_copy = pltpu.make_async_copy(w2_hbm, w2buf, sem_w.at[3])

    wq_copy.start()
    x_copy.start()
    gw_copy.start()
    w1_copy.start()
    w3_copy.start()
    w2_copy.start()
    for i in range(_NBUF):
        k_copy(i, i).start()
        v_copy(i, i).start()

    x_copy.wait()
    gw_copy.wait()
    x_row = xbuf[0]
    x8 = jnp.broadcast_to(x_row.astype(f32), (8, D)).astype(bf16)

    wq_copy.wait()
    for hp in range(H // 2):
        q2 = jnp.dot(x8, wqbuf[:, hp * 2 * DH:(hp + 1) * 2 * DH], preferred_element_type=f32)
        qbuf[2 * hp] = q2[:, :DH]
        qbuf[2 * hp + 1] = q2[:, DH:]

    w1_copy.wait()
    w3_copy.wait()
    gate = jnp.dot(x8, w1buf[...], preferred_element_type=f32)
    up = jnp.dot(x8, w3buf[...], preferred_element_type=f32)
    hid = (gate * jax.nn.sigmoid(gate) * up).astype(bf16)
    w2_copy.wait()
    b_out = jnp.dot(hid, w2buf[...], preferred_element_type=f32)
    gdot = jnp.sum(x_row.astype(f32) * gwbuf[...].astype(f32).reshape(1, D), axis=-1, keepdims=True)
    g = jax.nn.sigmoid(gdot)
    bbuf[0:8, :] = (1.0 - g) * b_out
    bbuf[8:16, :] = jnp.broadcast_to(g, (8, D))

    def head_body(h, carry):
        slot = h % _NBUF
        k_copy(h, slot).wait()
        q = qbuf[h].astype(bf16)
        s = jnp.dot(q, kbuf[slot], preferred_element_type=f32)

        @pl.when(h + _NBUF < H)
        def _():
            k_copy(h + _NBUF, slot).start()

        m = jnp.max(s, axis=-1, keepdims=True)
        p = jnp.exp((s - m) * scale)
        l = jnp.sum(p, axis=-1, keepdims=True)

        v_copy(h, slot).wait()
        acc = jnp.zeros((DH // 8, 8, _LANES), f32)
        for j in range(nblk):
            vj = vbuf[slot, :, j * _LANES:(j + 1) * _LANES].astype(f32).reshape(DH // 8, 8, _LANES)
            acc = acc + vj * p[None, :, j * _LANES:(j + 1) * _LANES]

        @pl.when(h + _NBUF < H)
        def _():
            v_copy(h + _NBUF, slot).start()

        @pl.when(h + _NBUF == H + 1)
        def _():
            for i in range(_WO_PIECES):
                wo_copy(i).start()

        o = jnp.sum(acc, axis=-1, keepdims=True) * (1.0 / l)[None]
        obuf[h] = jnp.broadcast_to(o, (DH // 8, 8, _LANES))
        return carry

    lax.fori_loop(0, H, head_body, 0)

    hpp = H // _WO_PIECES
    acc = jnp.zeros((8, D), f32)
    for i in range(_WO_PIECES):
        wo_copy(i).wait()

        def piece(t, a):
            h = i * hpp + t
            r0 = pl.multiple_of(h * DH, DH)
            w = wobuf[pl.ds(r0, DH), :].astype(f32).reshape(DH // 8, 8, D)
            ob = obuf[h]
            parts = []
            for c in range(D // _LANES):
                parts.append(jnp.sum(w[:, :, c * _LANES:(c + 1) * _LANES] * ob, axis=0))
            return a + jnp.concatenate(parts, axis=-1)

        acc = lax.fori_loop(0, hpp, piece, acc)
    a_out = jnp.sum(acc, axis=0, keepdims=True)
    res = bbuf[8:9, :] * a_out + bbuf[0:1, :]
    o_ref[0] = res.astype(o_ref.dtype)


@jax.jit
def pallas_gated_mix__sliding_block_cached__glu_gated_swiglu__decode_kernel(
    A_x: jax.Array,
    A_k_cache: jax.Array,
    A_v_cache: jax.Array,
    A_wq: jax.Array,
    A_wo: jax.Array,
    B_x: jax.Array,
    B_w1: jax.Array,
    B_w3: jax.Array,
    B_w2: jax.Array,
    gate_w: jax.Array,
):
    B, Sq, D = A_x.shape
    _, H, SK, DH = A_k_cache.shape
    assert B == 1 and Sq == 1
    assert A_wq.shape == (D, H * DH)
    F = B_w1.shape[1]
    W = min(4096, max(256, SK // 4))
    bf16 = jnp.bfloat16
    f32 = jnp.float32

    kt = jnp.swapaxes(A_k_cache, 2, 3)
    vt = jnp.swapaxes(A_v_cache, 2, 3)

    any_spec = pl.BlockSpec(memory_space=pl.ANY)
    kern = functools.partial(_kernel, H=H, DH=DH, SK=SK, W=W, D=D, F=F)
    return pl.pallas_call(
        kern,
        in_specs=[any_spec] * 9,
        out_specs=pl.BlockSpec(memory_space=pltpu.VMEM),
        out_shape=jax.ShapeDtypeStruct((B, Sq, D), A_x.dtype),
        scratch_shapes=[
            pltpu.VMEM((1, 1, D), bf16),
            pltpu.VMEM((D,), bf16),
            pltpu.VMEM((D, H * DH), bf16),
            pltpu.VMEM((H * DH, D), bf16),
            pltpu.VMEM((D, F), bf16),
            pltpu.VMEM((D, F), bf16),
            pltpu.VMEM((F, D), bf16),
            pltpu.VMEM((_NBUF, DH, W), bf16),
            pltpu.VMEM((_NBUF, DH, W), bf16),
            pltpu.VMEM((H, 8, DH), f32),
            pltpu.VMEM((H, DH // 8, 8, _LANES), f32),
            pltpu.VMEM((16, D), f32),
            pltpu.SemaphoreType.DMA((2,)),
            pltpu.SemaphoreType.DMA((4,)),
            pltpu.SemaphoreType.DMA((_NBUF,)),
            pltpu.SemaphoreType.DMA((_NBUF,)),
            pltpu.SemaphoreType.DMA((_WO_PIECES,)),
        ],
        compiler_params=pltpu.CompilerParams(vmem_limit_bytes=100 * 1024 * 1024),
    )(A_x, gate_w, A_wq, kt, vt, A_wo, B_w1, B_w3, B_w2)
```

```python
import functools

import jax
import jax.numpy as jnp
from jax import lax
import jax.experimental.pallas as pl
import jax.experimental.pallas.tpu as pltpu

_LANES = 128
_SC = 1024
_G = 8


def _interleave(main, extra):
    n, m = len(main), len(extra)
    keyed = [((i + 0.5) / n, 0, p) for i, p in enumerate(main)]
    keyed += [((j + 0.5) / m, 1, p) for j, p in enumerate(extra)]
    keyed.sort(key=lambda t: (t[0], t[1]))
    return [p for _, _, p in keyed]


class _Sub:
    def __init__(self, sems, base):
        self.sems, self.base = sems, base

    @property
    def at(self):
        return self

    def __getitem__(self, i):
        return self.sems.at[self.base + i]


def _kernel(x_hbm, gw_hbm, wq_hbm, k_hbm, v_hbm, wo_hbm, w1_hbm, w3_hbm, w2_hbm,
            o_ref,
            xbuf, gwbuf, wqbuf, wobuf, w1buf, w3buf, w2buf, kbuf, vbuf,
            qbuf, gubuf, accbuf,
            sems,
            *, H, DH, SK, W, D, F):
    sem_small, sem_k, sem_v, sem_wq, sem_wo, sem_mlp = (_Sub(sems, b) for b in (0, 3, 4, 8, 9, 12))
    f32 = jnp.float32
    bf16 = jnp.bfloat16
    scale = DH ** -0.5
    s0 = SK - W
    nsw = W // _SC
    ntr = DH // 8
    GC = _G * DH
    NG = H // _G
    wq_tr = D // 8 // _G
    w2_rows = F // _G

    def cp(src, dst, sem):
        return pltpu.make_async_copy(src, dst, sem)

    def kv_pieces(src, buf, h, sem_of_sweep):
        return [(None, cp(src.at[0, h, pl.ds(d * 8, 8), pl.ds(s0 + s * _SC, _SC)],
                          buf.at[pl.ds(d * 8, 8), pl.ds(s * _SC, _SC)], sem_of_sweep(s)))
                for s in range(nsw) for d in range(ntr)]

    def start_all(pieces):
        for i, (cond, c) in enumerate(pieces):
            if cond is None:
                c.start(priority=i % 2)
            else:
                pl.when(cond)(functools.partial(c.start, priority=i % 2))

    def wait_region(ref, sem):
        pltpu.make_async_copy(ref, ref, sem).wait()

    def wq_info(j):
        g = jnp.minimum(j // _G + 1, NG - 1)
        r0 = pl.multiple_of((j % _G) * (wq_tr * 8), 8)
        return j < H - _G, g, r0

    def wq_share(j):
        cond, g, r0 = wq_info(j)
        c0 = pl.multiple_of(g * GC, _LANES)
        return [(cond, cp(wq_hbm.at[pl.ds(r0 + t * 8, 8), pl.ds(c0, GC)],
                          wqbuf.at[g % 2, pl.ds(r0 + t * 8, 8), :], sem_wq.at[0])) for t in range(wq_tr)]

    def wo_share(j, nsplit=1):
        r0 = pl.multiple_of(j * DH, DH)
        n = DH // 16
        return [(None, cp(wo_hbm.at[pl.ds(r0 + t * 16, 16), :], wobuf.at[pl.ds(t * 16, 16), :],
                          sem_wo.at[t * nsplit // n])) for t in range(n)]

    def mlp_share(j):
        r0 = pl.multiple_of((j % _G) * (wq_tr * 8), 8)
        r2 = pl.multiple_of((j % _G) * w2_rows, 16)
        c1, c3, c2 = j < _G, (j >= _G) & (j < 2 * _G), (j >= 2 * _G) & (j < 3 * _G)
        p1 = [(c1, cp(w1_hbm.at[pl.ds(r0 + t * 8, 8), :], w1buf.at[pl.ds(r0 + t * 8, 8), :], sem_mlp.at[0]))
              for t in range(wq_tr)]
        p3 = [(c3, cp(w3_hbm.at[pl.ds(r0 + t * 8, 8), :], w3buf.at[pl.ds(r0 + t * 8, 8), :], sem_mlp.at[1]))
              for t in range(wq_tr)]
        p2 = [(c2, cp(w2_hbm.at[pl.ds(r2 + t * 16, 16), :], w2buf.at[pl.ds(r2 + t * 16, 16), :], sem_mlp.at[2]))
              for t in range(w2_rows // 16)]
        return p1, p3, p2

    def issue_k(j):
        start_all(_interleave(kv_pieces(k_hbm, kbuf, j, lambda s: sem_k.at[0]), wq_share(j)))

    def issue_v(j):
        p1, p3, p2 = mlp_share(j)
        main = kv_pieces(v_hbm, vbuf, j, lambda s: sem_v.at[0])
        main = _interleave(main, wo_share(j))
        n = max(len(p1), len(p2))
        slots = [[p[t] for p in (p1, p3, p2) if t < len(p)] for t in range(n)]
        mixed = _interleave([[p] for p in main], slots)
        for i, grp in enumerate(mixed):
            for cond, c in grp:
                if cond is None:
                    c.start(priority=i % 2)
                else:
                    pl.when(cond)(functools.partial(c.start, priority=i % 2))

    def q_group(x8, g, slot):
        r = jnp.dot(x8, wqbuf[slot], preferred_element_type=f32)
        for i in range(_G):
            qbuf[g * _G + i] = r[:, i * DH:(i + 1) * DH]

    def scores(h):
        q = qbuf[h].astype(bf16)
        s = jnp.dot(q, kbuf[...], preferred_element_type=f32)
        m = jnp.max(s, axis=-1, keepdims=True)
        p = jnp.exp((s - m) * scale)
        l = jnp.sum(p, axis=-1, keepdims=True)
        return p, l

    def pv(acc, p, j0, j1):
        for j in range(j0, j1):
            vj = vbuf[:, j * _LANES:(j + 1) * _LANES].astype(f32).reshape(ntr, 8, _LANES)
            acc = acc + vj * p[None, :, j * _LANES:(j + 1) * _LANES]
        return acc

    def o_cols(acc, l):
        o = jnp.sum(acc, axis=-1, keepdims=True) * (1.0 / l)[None]
        return jnp.broadcast_to(o, (ntr, 8, _LANES))

    def wo_apply(ob, t0, t1):
        w = wobuf[t0 * 8:t1 * 8, :].astype(f32).reshape(t1 - t0, 8, D)
        parts = [jnp.sum(w[:, :, c * _LANES:(c + 1) * _LANES] * ob[t0:t1], axis=0) for c in range(D // _LANES)]
        return jnp.concatenate(parts, axis=-1)

    x_copy = cp(x_hbm, xbuf, sem_small.at[0])
    gw_copy = cp(gw_hbm, gwbuf, sem_small.at[1])
    ntq = D // 8
    order0 = [t for r in range(4) for t in range(r, ntq, 4)]
    start_all([(None, cp(wq_hbm.at[pl.ds(t * 8, 8), pl.ds(0, GC)], wqbuf.at[0, pl.ds(t * 8, 8), :], sem_small.at[2]))
               for t in order0] + [(None, x_copy), (None, gw_copy)])
    issue_k(0)
    x_copy.wait()
    gw_copy.wait()
    wait_region(wqbuf.at[0], sem_small.at[2])
    x_row = xbuf[0].astype(f32)
    x8 = jnp.broadcast_to(x_row, (8, D)).astype(bf16)
    q_group(x8, 0, 0)
    accbuf[...] = jnp.zeros(accbuf.shape, f32)

    def get_x8():
        return jnp.broadcast_to(xbuf[0].astype(f32), (8, D)).astype(bf16)

    def wait_k(h):
        wait_region(kbuf, sem_k.at[0])
        cond, g, r0 = wq_info(h)
        slot = g % 2

        @pl.when(cond)
        def _():
            wait_region(wqbuf.at[slot, pl.ds(r0, wq_tr * 8), :], sem_wq.at[0])

    def head_body(h, carry):
        issue_v(h)
        wait_k(h)
        p, l = scores(h)

        @pl.when((h % _G == _G - 1))
        def _():
            g = h // _G + 1
            q_group(get_x8(), g, g % 2)

        issue_k(h + 1)
        wait_region(vbuf, sem_v.at[0])
        wait_region(wobuf, sem_wo.at[0])
        acc = pv(jnp.zeros((ntr, 8, _LANES), f32), p, 0, W // _LANES)
        accbuf[...] += wo_apply(o_cols(acc, l), 0, ntr)

        @pl.when(h == _G - 1)
        def _():
            wait_region(w1buf, sem_mlp.at[0])
            gubuf[0:8, :] = jnp.dot(get_x8(), w1buf[...], preferred_element_type=f32)

        @pl.when(h == 2 * _G - 1)
        def _():
            wait_region(w3buf, sem_mlp.at[1])
            up = jnp.dot(get_x8(), w3buf[...], preferred_element_type=f32)
            gate = gubuf[0:8, :]
            gubuf[0:8, :] = gate * jax.nn.sigmoid(gate) * up

        @pl.when(h == 3 * _G - 1)
        def _():
            wait_region(w2buf, sem_mlp.at[2])
            b_out = jnp.dot(gubuf[0:8, :].astype(bf16), w2buf[...], preferred_element_type=f32)
            gdot = jnp.sum(xbuf[0].astype(f32) * gwbuf[...].astype(f32).reshape(1, D), axis=-1, keepdims=True)
            g = jax.nn.sigmoid(gdot)
            gubuf[0:8, 0:D] = (1.0 - g) * b_out
            gubuf[8:16, 0:D] = jnp.broadcast_to(g, (8, D))
        return carry

    lax.fori_loop(0, H - 1, head_body, 0)

    h = H - 1
    nsplit = 3
    start_all(kv_pieces(v_hbm, vbuf, h, lambda s: sem_v.at[s]) + wo_share(h, nsplit))
    wait_region(kbuf, sem_k.at[0])
    p, l = scores(h)
    acc = jnp.zeros((ntr, 8, _LANES), f32)
    bps = _SC // _LANES
    for s in range(nsw):
        wait_region(vbuf.at[:, pl.ds(s * _SC, _SC)], sem_v.at[s])
        acc = pv(acc, p, s * bps, (s + 1) * bps)
    ob = o_cols(acc, l)
    a8 = accbuf[...]
    tps = ntr // nsplit
    for i in range(nsplit):
        wait_region(wobuf.at[pl.ds(i * tps * 8, tps * 8), :], sem_wo.at[i])
        a8 = a8 + wo_apply(ob, i * tps, (i + 1) * tps)
    a_out = jnp.sum(a8, axis=0, keepdims=True)
    res = gubuf[8:9, 0:D] * a_out + gubuf[0:1, 0:D]
    o_ref[0] = res.astype(o_ref.dtype)


@jax.jit
def pallas_gated_mix__sliding_block_cached__glu_gated_swiglu__decode_kernel(
    A_x: jax.Array,
    A_k_cache: jax.Array,
    A_v_cache: jax.Array,
    A_wq: jax.Array,
    A_wo: jax.Array,
    B_x: jax.Array,
    B_w1: jax.Array,
    B_w3: jax.Array,
    B_w2: jax.Array,
    gate_w: jax.Array,
):
    B, Sq, D = A_x.shape
    _, H, SK, DH = A_k_cache.shape
    assert B == 1 and Sq == 1
    assert A_wq.shape == (D, H * DH)
    F = B_w1.shape[1]
    W = min(4096, max(256, SK // 4))
    bf16 = jnp.bfloat16
    f32 = jnp.float32

    kt = jnp.swapaxes(A_k_cache, 2, 3)
    vt = jnp.swapaxes(A_v_cache, 2, 3)

    any_spec = pl.BlockSpec(memory_space=pl.ANY)
    kern = functools.partial(_kernel, H=H, DH=DH, SK=SK, W=W, D=D, F=F)
    return pl.pallas_call(
        kern,
        in_specs=[any_spec] * 9,
        out_specs=pl.BlockSpec(memory_space=pltpu.VMEM),
        out_shape=jax.ShapeDtypeStruct((B, Sq, D), A_x.dtype),
        scratch_shapes=[
            pltpu.VMEM((1, 1, D), bf16),
            pltpu.VMEM((D,), bf16),
            pltpu.VMEM((2, D, _G * DH), bf16),
            pltpu.VMEM((DH, D), bf16),
            pltpu.VMEM((D, F), bf16),
            pltpu.VMEM((D, F), bf16),
            pltpu.VMEM((F, D), bf16),
            pltpu.VMEM((DH, W), bf16),
            pltpu.VMEM((DH, W), bf16),
            pltpu.VMEM((H, 8, DH), f32),
            pltpu.VMEM((16, F), f32),
            pltpu.VMEM((8, D), f32),
            pltpu.SemaphoreType.DMA((15,)),
        ],
        compiler_params=pltpu.CompilerParams(vmem_limit_bytes=64 * 1024 * 1024,
                                             disable_bounds_checks=True,
                                             disable_semaphore_checks=True),
    )(A_x, gate_w, A_wq, kt, vt, A_wo, B_w1, B_w3, B_w2)
```

```python
import functools

import jax
import jax.numpy as jnp
from jax import lax
import jax.experimental.pallas as pl
import jax.experimental.pallas.tpu as pltpu

_LANES = 128
CFG = dict(
    kv_split=(6, 8, 8, 10),
    last_split=(6, 8, 8, 8, 2),
    wq_st=24,
    rest_st=24,
    wo_rows=24, w2_rows=24,
    tail_rows=192,
    tail_split=3,
    first_rest=80,
)


def _spans(split):
    out, c = [], 0
    for z in split:
        out.append((c * _LANES, z * _LANES))
        c += z
    return out


def _strided(items, st):
    return [items[i] for r in range(st) for i in range(r, len(items), st)]


def _kernel(x_hbm, gw_hbm, wq_hbm, k_hbm, v_hbm, wo_hbm, w1_hbm, w3_hbm, w2_hbm,
            o_ref,
            xbuf, gwbuf, wqbuf, wobuf, w1buf, w3buf, w2buf, kbuf, vbuf,
            qbuf, gubuf, accbuf,
            sems,
            *, H, DH, SK, W, D, F):
    f32 = jnp.float32
    bf16 = jnp.bfloat16
    scale = DH ** -0.5
    s0 = SK - W
    ntr = DH // 8
    NOC = CFG.get("nocompute", False)
    tail_rows, nsplit = CFG["tail_rows"], CFG["tail_split"]
    S_X, S_GW, S_WQ, S_W1, S_W3, S_W2, S_WO, S_K, S_V, S_WOT = 0, 1, 2, 3, 4, 5, 6, 7, 9, 11
    S_VL = S_WOT + nsplit

    def cp(src, dst, sem):
        return pltpu.make_async_copy(src, dst, sems.at[sem])

    def kv_pieces(src, buf, h, split, sem_of_sweep):
        assert sum(split) * _LANES == W
        return [[cp(src.at[0, h, pl.ds(d * 8, 8), pl.ds(s0 + c, z)],
                    buf.at[pl.ds(d * 8, 8), pl.ds(c, z)], sem_of_sweep(s))]
                for s, (c, z) in enumerate(_spans(split)) for d in range(ntr)]

    def start_all(slots):
        for i, grp in enumerate(slots):
            for c in grp:
                c.start(priority=i % 2)

    def wait_region(ref, sem):
        pltpu.make_async_copy(ref, ref, sems.at[sem]).wait()

    def rect(src, dst, r, nr, c, nc, sem):
        return cp(src.at[pl.ds(r, nr), pl.ds(c, nc)], dst.at[pl.ds(r, nr), pl.ds(c, nc)], sem)

    def rows(src, dst, r0, r1, rr, sem):
        assert (r1 - r0) % rr == 0
        return [[cp(src.at[pl.ds(r, rr), :], dst.at[pl.ds(r, rr), :], sem)] for r in range(r0, r1, rr)]

    def delay():
        n = CFG.get("delay", 0)
        a0 = accbuf[:, 0:_LANES]
        return lax.fori_loop(0, n, lambda i, a: a * 1.0001 + 0.5, a0) if n else a0

    def scores(h, kb):
        if NOC:
            a = delay()
            return jnp.ones((8, W), f32), a[:, 0:1]
        q = qbuf[h].astype(bf16)
        s = jnp.dot(q, kb[...], preferred_element_type=f32)
        m = jnp.max(s, axis=-1, keepdims=True)
        p = jnp.exp((s - m) * scale)
        l = jnp.sum(p, axis=-1, keepdims=True)
        return p, l

    def pv(vb, acc, p, j0, j1):
        if NOC:
            if j1 - j0 == W // _LANES:
                return acc + delay()[None]
            return acc
        for j in range(j0, j1):
            vj = vb[:, j * _LANES:(j + 1) * _LANES].astype(f32).reshape(ntr, 8, _LANES)
            acc = acc + vj * p[None, :, j * _LANES:(j + 1) * _LANES]
        return acc

    def o_cols(acc, l):
        o = jnp.sum(acc, axis=-1, keepdims=True) * (1.0 / l)[None]
        return jnp.broadcast_to(o, (ntr, 8, _LANES))

    def wo_apply(ob, r0, t0, t1):
        if NOC:
            return jnp.concatenate([ob[0]] * (D // _LANES), axis=-1)
        w = wobuf[pl.ds(r0 + t0 * 8, (t1 - t0) * 8), :].astype(f32).reshape(t1 - t0, 8, D)
        parts = [jnp.sum(w[:, :, c * _LANES:(c + 1) * _LANES] * ob[t0:t1], axis=0) for c in range(D // _LANES)]
        return jnp.concatenate(parts, axis=-1)

    def get_x8():
        return jnp.broadcast_to(xbuf[0].astype(f32), (8, D)).astype(bf16)

    x_copy = cp(x_hbm, xbuf, S_X)
    gw_copy = cp(gw_hbm, gwbuf, S_GW)
    L = _LANES
    wq_blocks = []
    ntq = D // 8
    if CFG.get("wq_aligned", True):
        for t in range(ntq):
            first = [rect(wq_hbm, wqbuf, t * 8, 8, 0, 14 * L, S_WQ)]
            if t > 0:
                first = [rect(wq_hbm, wqbuf, (t - 1) * 8, 8, 46 * L, 2 * L, S_WQ)] + first
            wq_blocks.append(first)
            wq_blocks.append([rect(wq_hbm, wqbuf, t * 8, 8, 14 * L, 16 * L, S_WQ)])
            last = [rect(wq_hbm, wqbuf, t * 8, 8, 30 * L, (16 if t < ntq - 1 else 18) * L, S_WQ)]
            wq_blocks.append(last)
    else:
        for t in range(ntq):
            for c in range(3):
                wq_blocks.append([rect(wq_hbm, wqbuf, t * 8, 8, c * 16 * L, 16 * L, S_WQ)])
    HD = H * DH
    rest = (rows(wo_hbm, wobuf, 0, HD - tail_rows, CFG["wo_rows"], S_WO) + rows(w1_hbm, w1buf, 0, D, 8, S_W1)
            + rows(w3_hbm, w3buf, 0, D, 8, S_W3) + rows(w2_hbm, w2buf, 0, F, CFG["w2_rows"], S_W2))
    rest = _strided(rest, CFG["rest_st"])
    n1 = CFG["first_rest"]
    start_all(_strided(wq_blocks, CFG["wq_st"]) + [[x_copy], [gw_copy]] + rest[:n1])
    accbuf[...] = jnp.zeros(accbuf.shape, f32)
    x_copy.wait()
    gw_copy.wait()
    wait_region(wqbuf, S_WQ)
    if not NOC:
        x8 = get_x8()
        for hp in range(H // 2):
            q2 = jnp.dot(x8, wqbuf[:, hp * 2 * DH:(hp + 1) * 2 * DH], preferred_element_type=f32)
            qbuf[2 * hp] = q2[:, :DH]
            qbuf[2 * hp + 1] = q2[:, DH:]
    KS = CFG["kv_split"]
    start_all(rest[n1:] + kv_pieces(k_hbm, kbuf.at[0], 0, KS, lambda s: S_K))
    wait_region(wobuf.at[pl.ds(0, HD - tail_rows), :], S_WO)
    wait_region(w1buf, S_W1)
    wait_region(w3buf, S_W3)
    wait_region(w2buf, S_W2)
    if not NOC:
        gubuf[0:8, :] = jnp.dot(get_x8(), w1buf[...], preferred_element_type=f32)
    start_all(kv_pieces(v_hbm, vbuf.at[0], 0, KS, lambda s: S_V))
    if not NOC:
        up = jnp.dot(get_x8(), w3buf[...], preferred_element_type=f32)
        gate = gubuf[0:8, :]
        gubuf[0:8, :] = gate * jax.nn.sigmoid(gate) * up

    def attend(h, slot):
        wait_region(vbuf.at[slot], S_V + slot)

    def head_body(h, carry):
        slot = h % 2
        nslot = 1 - slot
        start_all(kv_pieces(k_hbm, kbuf.at[nslot], h + 1, KS, lambda s: S_K + nslot))
        wait_region(kbuf.at[slot], S_K + slot)
        p, l = scores(h, kbuf.at[slot])

        @pl.when(h == 0)
        def _():
            if NOC:
                return
            b_out = jnp.dot(gubuf[0:8, :].astype(bf16), w2buf[...], preferred_element_type=f32)
            gdot = jnp.sum(xbuf[0].astype(f32) * gwbuf[...].astype(f32).reshape(1, D), axis=-1, keepdims=True)
            g = jax.nn.sigmoid(gdot)
            gubuf[0:8, 0:D] = (1.0 - g) * b_out
            gubuf[8:16, 0:D] = jnp.broadcast_to(g, (8, D))

        @pl.when(h < H - 2)
        def _():
            start_all(kv_pieces(v_hbm, vbuf.at[nslot], h + 1, KS, lambda s: S_V + nslot))

        @pl.when(h == H - 2)
        def _():
            start_all(last_batch())

        wait_region(vbuf.at[slot], S_V + slot)
        acc = pv(vbuf.at[slot], jnp.zeros((ntr, 8, _LANES), f32), p, 0, W // _LANES)
        accbuf[...] += wo_apply(o_cols(acc, l), pl.multiple_of(h * DH, DH), 0, ntr)
        return carry

    lslot = (H - 1) % 2
    tr = tail_rows // nsplit

    def last_batch():
        tail = []
        if tail_rows:
            assert tail_rows % nsplit == 0 and tr % 8 == 0 and tail_rows <= DH
            for i in range(nsplit):
                a = HD - tail_rows + i * tr
                tail += rows(wo_hbm, wobuf, a, a + tr, min(tr, CFG.get("tail_rr", 16)), S_WOT + i)
        return kv_pieces(v_hbm, vbuf.at[lslot], H - 1, CFG["last_split"], lambda s: S_VL + s) + tail

    lax.fori_loop(0, H - 1, head_body, 0)

    h = H - 1
    wait_region(kbuf.at[lslot], S_K + lslot)
    p, l = scores(h, kbuf.at[lslot])
    acc = jnp.zeros((ntr, 8, _LANES), f32)
    for s, (c, z) in enumerate(_spans(CFG["last_split"])):
        wait_region(vbuf.at[lslot, :, pl.ds(c, z)], S_VL + s)
        acc = pv(vbuf.at[lslot], acc, p, c // _LANES, (c + z) // _LANES)
    ob = o_cols(acc, l)
    a8 = accbuf[...]
    t_res = (DH - tail_rows) // 8
    if t_res:
        a8 = a8 + wo_apply(ob, h * DH, 0, t_res)
    if tail_rows:
        for i in range(nsplit):
            a = HD - tail_rows + i * tr
            wait_region(wobuf.at[pl.ds(a, tr), :], S_WOT + i)
            a8 = a8 + wo_apply(ob, h * DH, t_res + i * tr // 8, t_res + (i + 1) * tr // 8)
    a_out = jnp.sum(a8, axis=0, keepdims=True)
    res = gubuf[8:9, 0:D] * a_out + gubuf[0:1, 0:D]
    o_ref[0] = res.astype(o_ref.dtype)


@jax.jit
def pallas_gated_mix__sliding_block_cached__glu_gated_swiglu__decode_kernel(
    A_x: jax.Array,
    A_k_cache: jax.Array,
    A_v_cache: jax.Array,
    A_wq: jax.Array,
    A_wo: jax.Array,
    B_x: jax.Array,
    B_w1: jax.Array,
    B_w3: jax.Array,
    B_w2: jax.Array,
    gate_w: jax.Array,
):
    B, Sq, D = A_x.shape
    _, H, SK, DH = A_k_cache.shape
    assert B == 1 and Sq == 1
    assert A_wq.shape == (D, H * DH)
    F = B_w1.shape[1]
    W = min(4096, max(256, SK // 4))
    bf16 = jnp.bfloat16
    f32 = jnp.float32

    kt = jnp.swapaxes(A_k_cache, 2, 3)
    vt = jnp.swapaxes(A_v_cache, 2, 3)

    any_spec = pl.BlockSpec(memory_space=pl.ANY)
    kern = functools.partial(_kernel, H=H, DH=DH, SK=SK, W=W, D=D, F=F)
    return pl.pallas_call(
        kern,
        in_specs=[any_spec] * 9,
        out_specs=pl.BlockSpec(memory_space=pltpu.VMEM),
        out_shape=jax.ShapeDtypeStruct((B, Sq, D), A_x.dtype),
        scratch_shapes=[
            pltpu.VMEM((1, 1, D), bf16),
            pltpu.VMEM((D,), bf16),
            pltpu.VMEM((D, H * DH), bf16),
            pltpu.VMEM((H * DH, D), bf16),
            pltpu.VMEM((D, F), bf16),
            pltpu.VMEM((D, F), bf16),
            pltpu.VMEM((F, D), bf16),
            pltpu.VMEM((2, DH, W), bf16),
            pltpu.VMEM((2, DH, W), bf16),
            pltpu.VMEM((H, 8, DH), f32),
            pltpu.VMEM((16, F), f32),
            pltpu.VMEM((8, D), f32),
            pltpu.SemaphoreType.DMA((11 + CFG["tail_split"] + len(CFG["last_split"]),)),
        ],
        compiler_params=pltpu.CompilerParams(vmem_limit_bytes=64 * 1024 * 1024,
                                             disable_bounds_checks=True,
                                             disable_semaphore_checks=True),
    )(A_x, gate_w, A_wq, kt, vt, A_wo, B_w1, B_w3, B_w2)
```

```python
import functools

import jax
import jax.numpy as jnp
from jax import lax
import jax.experimental.pallas as pl
import jax.experimental.pallas.tpu as pltpu

_L = 128
CFG = dict(
    kv_split=(6, 8, 4, 4, 10),
    last_split=(6, 8, 8, 6, 4),
    hold=(16, 6, 2),
    hold_rr=16,
    wq_st=24, rest_st=34, wo_rows=24, w2_rows=24, first_rest=80, cuts=(48,),
)


def _spans(split):
    out, c = [], 0
    for z in split:
        out.append((c, z))
        c += z
    return out


def _strided(items, st):
    return [items[i] for r in range(st) for i in range(r, len(items), st)]


def _kernel(x_hbm, gw_hbm, wq_hbm, k_hbm, v_hbm, wo_hbm, w1_hbm, w3_hbm, w2_hbm,
            o_ref,
            xbuf, gwbuf, wqbuf, wobuf, w1buf, w3buf, w2buf, kbuf, vbuf,
            qbuf, hbuf, gbuf, accbuf,
            sems,
            *, H, DH, SK, W, D, F):
    f32 = jnp.float32
    bf16 = jnp.bfloat16
    scale = DH ** -0.5
    s0 = SK - W
    ntr = DH // 8
    HD = H * DH
    KS, LS, HOLD = CFG["kv_split"], CFG["last_split"], CFG["hold"]
    assert sum(KS) * _L == W and sum(LS) * _L == W
    S_X, S_GW, S_WQ, S_W1, S_W3, S_W2, S_WO, S_K, S_V, S_VL = 0, 1, 2, 3, 4, 5, 6, 7, 9, 11
    S_HOLD = S_VL + len(LS)
    ne = ntr - sum(HOLD)
    wo_early = HD - sum(HOLD) * 8

    def start_all(slots, first=0):
        for i, slot in enumerate(slots):
            for src, dst, sem in slot:
                pltpu.make_async_copy(src, dst, sems.at[sem]).start(priority=(first + i) % 2)

    def wait_for(ref, sem):
        pltpu.make_async_copy(ref, ref, sems.at[sem]).wait()

    def kv_jobs(src, buf, h, split, sem_of):
        return [[(src.at[0, h, pl.ds(d * 8, 8), pl.ds(s0 + c * _L, z * _L)],
                  buf.at[pl.ds(d * 8, 8), pl.ds(c * _L, z * _L)], sem_of(s))]
                for s, (c, z) in enumerate(_spans(split)) for d in range(ntr)]

    def rect(src, dst, r, nr, c, nc, sem):
        return (src.at[pl.ds(r, nr), pl.ds(c * _L, nc * _L)], dst.at[pl.ds(r, nr), pl.ds(c * _L, nc * _L)], sem)

    def row_jobs(src, dst, r0, r1, rr, sem):
        return [[(src.at[pl.ds(r, min(rr, r1 - r)), :], dst.at[pl.ds(r, min(rr, r1 - r)), :], sem)]
                for r in range(r0, r1, rr)]

    def scores(h, kb):
        q = qbuf[h].astype(bf16)
        s = jnp.dot(q, kb[...], preferred_element_type=f32)
        m = jnp.max(s, axis=-1, keepdims=True)
        p = jnp.exp((s - m) * scale)
        return p, jnp.sum(p, axis=-1, keepdims=True)

    def pv(vb, acc, p, j0, j1):
        for j in range(j0, j1):
            vj = vb[:, j * _L:(j + 1) * _L].astype(f32).reshape(ntr, 8, _L)
            acc = acc + vj * p[None, :, j * _L:(j + 1) * _L]
        return acc

    def o_cols(acc, l):
        return jnp.sum(acc, axis=-1, keepdims=True) * (gbuf[...] / l)[None]

    def wo_apply(ob, r0):
        n = ob.shape[0]
        w = wobuf[pl.ds(r0, n * 8), :].astype(f32).reshape(n, 8, D)
        return [jnp.sum(w[:, :, c * _L:(c + 1) * _L] * ob, axis=0) for c in range(D // _L)]

    ntq = D // 8
    wq_slots = []
    for t in range(ntq):
        first = [rect(wq_hbm, wqbuf, t * 8, 8, 0, 14, S_WQ)]
        if t > 0:
            first = [rect(wq_hbm, wqbuf, (t - 1) * 8, 8, 46, 2, S_WQ)] + first
        wq_slots.append(first)
        wq_slots.append([rect(wq_hbm, wqbuf, t * 8, 8, 14, 16, S_WQ)])
        wq_slots.append([rect(wq_hbm, wqbuf, t * 8, 8, 30, 16 if t < ntq - 1 else 18, S_WQ)])
    rest = (row_jobs(wo_hbm, wobuf, 0, wo_early, CFG["wo_rows"], S_WO) + row_jobs(w1_hbm, w1buf, 0, D, 8, S_W1)
            + row_jobs(w3_hbm, w3buf, 0, D, 8, S_W3) + row_jobs(w2_hbm, w2buf, 0, F, CFG["w2_rows"], S_W2))
    rest = _strided(rest, CFG["rest_st"])
    n1 = CFG["first_rest"]
    start_all(_strided(wq_slots, CFG["wq_st"]) + [[(x_hbm, xbuf, S_X)], [(gw_hbm, gwbuf, S_GW)]] + rest[:n1])
    wait_for(xbuf, S_X)
    wait_for(gwbuf, S_GW)
    wait_for(wqbuf, S_WQ)
    x_row = xbuf[0].astype(f32)
    x8 = jnp.broadcast_to(x_row, (8, D)).astype(bf16)
    gdot = jnp.sum(x_row * gwbuf[...].astype(f32).reshape(1, D), axis=-1, keepdims=True)
    gbuf[...] = jnp.broadcast_to(jax.nn.sigmoid(gdot), gbuf.shape)
    for hp in range(H // 2):
        q2 = jnp.dot(x8, wqbuf[:, hp * 2 * DH:(hp + 1) * 2 * DH], preferred_element_type=f32)
        qbuf[2 * hp] = q2[:, :DH]
        qbuf[2 * hp + 1] = q2[:, DH:]
    start_all(rest[n1:])
    start_all(kv_jobs(k_hbm, kbuf.at[0], 0, KS, lambda s: S_K))
    wait_for(wobuf.at[pl.ds(0, wo_early), :], S_WO)
    wait_for(w1buf, S_W1)
    wait_for(w3buf, S_W3)
    wait_for(w2buf, S_W2)
    gate = jnp.dot(x8, w1buf[...], preferred_element_type=f32)
    start_all(kv_jobs(v_hbm, vbuf.at[0], 0, KS, lambda s: S_V))
    up = jnp.dot(x8, w3buf[...], preferred_element_type=f32)
    hbuf[...] = gate * jax.nn.sigmoid(gate) * up

    lslot = (H - 1) % 2

    def last_jobs():
        jobs = kv_jobs(v_hbm, vbuf.at[lslot], H - 1, LS, lambda s: S_VL + s)
        assert len(jobs) % 2 == 0
        for g, (t0, n) in enumerate(_spans(HOLD)):
            r0 = wo_early + t0 * 8
            for job in row_jobs(wo_hbm, wobuf, r0, r0 + n * 8, CFG["hold_rr"], S_HOLD + g):
                jobs += [[], job]
        return jobs

    def head_body(h, carry):
        slot = h % 2
        nslot = 1 - slot
        start_all(kv_jobs(k_hbm, kbuf.at[nslot], h + 1, KS, lambda s: S_K + nslot))
        wait_for(kbuf.at[slot], S_K + slot)
        p, l = scores(h, kbuf.at[slot])

        @pl.when(h == 0)
        def _():
            b_out = jnp.dot(hbuf[...].astype(bf16), w2buf[...], preferred_element_type=f32)
            row0 = lax.broadcasted_iota(jnp.int32, (8, D), 0) == 0
            accbuf[...] = jnp.where(row0, (1.0 - gbuf[:, 0:1]) * b_out, 0.0)

        @pl.when(h < H - 2)
        def _():
            start_all(kv_jobs(v_hbm, vbuf.at[nslot], h + 1, KS, lambda s: S_V + nslot))

        @pl.when(h == H - 2)
        def _():
            start_all(last_jobs()[:CFG["cuts"][0]])

        wait_for(vbuf.at[slot], S_V + slot)
        acc = pv(vbuf.at[slot], jnp.zeros((ntr, 8, _L), f32), p, 0, W // _L)
        parts = wo_apply(o_cols(acc, l), pl.multiple_of(h * DH, DH))
        accbuf[...] += jnp.concatenate(parts, axis=-1)
        return carry

    lax.fori_loop(0, H - 1, head_body, 0)

    h = H - 1
    lj = last_jobs()
    cuts = list(CFG["cuts"]) + [len(lj)] * (len(LS) + 3)

    def issue_part(i):
        start_all(lj[cuts[i - 1]:cuts[i]], first=cuts[i - 1])

    issue_part(1)
    vb = vbuf.at[lslot]
    wait_for(kbuf.at[lslot], S_K + lslot)
    p, l = scores(h, kbuf.at[lslot])
    acc = jnp.zeros((ntr, 8, _L), f32)
    for s, (c, z) in enumerate(_spans(LS)):
        issue_part(2 + s)
        assert cuts[2 + s] >= (s + 1) * ntr and cuts[1 + len(LS)] == len(lj)
        wait_for(vb.at[:, pl.ds(c * _L, z * _L)], S_VL + s)
        acc = pv(vb, acc, p, c, c + z)
    ob = o_cols(acc, l)
    tot = accbuf[...]
    tot = [tot[:, c * _L:(c + 1) * _L] for c in range(D // _L)]
    if ne:
        tot = [a + b for a, b in zip(tot, wo_apply(ob[:ne], h * DH))]
    for g, (t0, n) in enumerate(_spans(HOLD)):
        r0 = wo_early + t0 * 8
        wait_for(wobuf.at[pl.ds(r0, n * 8), :], S_HOLD + g)
        tot = [a + b for a, b in zip(tot, wo_apply(ob[ne + t0:ne + t0 + n], r0))]
    for c in range(D // _L):
        o_ref[0, :, c * _L:(c + 1) * _L] = jnp.sum(tot[c], axis=0, keepdims=True).astype(o_ref.dtype)


@jax.jit
def pallas_gated_mix__sliding_block_cached__glu_gated_swiglu__decode_kernel(
    A_x: jax.Array,
    A_k_cache: jax.Array,
    A_v_cache: jax.Array,
    A_wq: jax.Array,
    A_wo: jax.Array,
    B_x: jax.Array,
    B_w1: jax.Array,
    B_w3: jax.Array,
    B_w2: jax.Array,
    gate_w: jax.Array,
):
    B, Sq, D = A_x.shape
    _, H, SK, DH = A_k_cache.shape
    assert B == 1 and Sq == 1
    assert A_wq.shape == (D, H * DH)
    F = B_w1.shape[1]
    W = min(4096, max(256, SK // 4))
    bf16 = jnp.bfloat16
    f32 = jnp.float32

    kt = jnp.swapaxes(A_k_cache, 2, 3)
    vt = jnp.swapaxes(A_v_cache, 2, 3)

    any_spec = pl.BlockSpec(memory_space=pl.ANY)
    kern = functools.partial(_kernel, H=H, DH=DH, SK=SK, W=W, D=D, F=F)
    return pl.pallas_call(
        kern,
        in_specs=[any_spec] * 9,
        out_specs=pl.BlockSpec(memory_space=pltpu.VMEM),
        out_shape=jax.ShapeDtypeStruct((B, Sq, D), A_x.dtype),
        scratch_shapes=[
            pltpu.VMEM((1, 1, D), bf16),
            pltpu.VMEM((D,), bf16),
            pltpu.VMEM((D, H * DH), bf16),
            pltpu.VMEM((H * DH, D), bf16),
            pltpu.VMEM((D, F), bf16),
            pltpu.VMEM((D, F), bf16),
            pltpu.VMEM((F, D), bf16),
            pltpu.VMEM((2, DH, W), bf16),
            pltpu.VMEM((2, DH, W), bf16),
            pltpu.VMEM((H, 8, DH), f32),
            pltpu.VMEM((8, F), f32),
            pltpu.VMEM((8, _L), f32),
            pltpu.VMEM((8, D), f32),
            pltpu.SemaphoreType.DMA((11 + len(CFG["last_split"]) + len(CFG["hold"]),)),
        ],
        compiler_params=pltpu.CompilerParams(vmem_limit_bytes=64 * 1024 * 1024,
                                             disable_bounds_checks=True,
                                             disable_semaphore_checks=True),
    )(A_x, gate_w, A_wq, kt, vt, A_wo, B_w1, B_w3, B_w2)
```

```python
import functools

import jax
import jax.numpy as jnp
from jax import lax
import jax.experimental.pallas as pl
import jax.experimental.pallas.tpu as pltpu

_L = 128
_KV_SPLIT = (6, 8, 4, 4, 10)
_LAST_SPLIT = (6, 8, 8, 6, 4)
_HOLD = (16, 6, 2)
_RUN = 16
_WQ_STRIDE = 24
_REST_STRIDE = 8
_REST_AHEAD = 48
_LAST_AHEAD = 48


def _spans(split):
    out, c = [], 0
    for z in split:
        out.append((c, z))
        c += z
    return out


def _strided(items, st):
    return [items[i] for r in range(st) for i in range(r, len(items), st)]


def _kernel(x_hbm, gw_hbm, wq_hbm, k_hbm, v_hbm, wo_hbm, w1_hbm, w3_hbm, w2_hbm,
            o_ref,
            xbuf, gwbuf, wqbuf, wobuf, w1buf, w3buf, w2buf, kbuf, vbuf,
            qbuf, hbuf, gbuf, accbuf,
            sems,
            *, H, DH, SK, W, D, F):
    f32 = jnp.float32
    bf16 = jnp.bfloat16
    scale = DH ** -0.5
    s0 = SK - W
    ntr = DH // 8
    ncb = D // _L
    S_X, S_GW, S_WQ, S_W1, S_W3, S_W2, S_WO, S_K, S_V, S_VL = 0, 1, 2, 3, 4, 5, 6, 7, 9, 11
    S_HOLD = S_VL + len(_LAST_SPLIT)
    wo_early = (H - 1) * DH

    def start_all(slots, first=0):
        for i, slot in enumerate(slots):
            for src, dst, sem in slot:
                pltpu.make_async_copy(src, dst, sems.at[sem]).start(priority=(first + i) % 2)

    def wait_for(ref, sem):
        pltpu.make_async_copy(ref, ref, sems.at[sem]).wait()

    def kv_jobs(src, buf, h, split, sem_of):
        return [[(src.at[0, h, pl.ds(d * 8, 8), pl.ds(s0 + c * _L, z * _L)],
                  buf.at[pl.ds(d * 8, 8), pl.ds(c * _L, z * _L)], sem_of(s))]
                for s, (c, z) in enumerate(_spans(split)) for d in range(ntr)]

    def rect(src, dst, t, nt, c, nc, sem):
        idx = (pl.ds(t * 8, nt * 8), pl.ds(c * _L, nc * _L))
        return (src.at[idx], dst.at[idx], sem)

    def run_slots(src, dst, nrows, first_cut, sem):
        cw = src.shape[1] // _L
        nt = nrows // 8 * cw
        cuts = sorted(set([0, nt] + list(range(first_cut, nt, _RUN))))
        slots = []
        for s, e in zip(cuts[:-1], cuts[1:]):
            slot = []
            if s % cw:
                m = min(e, (s // cw + 1) * cw)
                slot.append(rect(src, dst, s // cw, 1, s % cw, m - s, sem))
                s = m
            if e - s >= cw:
                n = (e - s) // cw
                slot.append(rect(src, dst, s // cw, n, 0, cw, sem))
                s += n * cw
            if e > s:
                slot.append(rect(src, dst, s // cw, 1, 0, e - s, sem))
            slots.append(slot)
        return slots

    def scores(h, kb):
        q = qbuf[h].astype(bf16)
        s = jnp.dot(q, kb[...], preferred_element_type=f32)
        m = jnp.max(s, axis=-1, keepdims=True)
        p = jnp.exp((s - m) * scale)
        return p, jnp.sum(p, axis=-1, keepdims=True)

    def pv(vb, acc, p, j0, j1):
        for j in range(j0, j1):
            vj = vb[:, j * _L:(j + 1) * _L].astype(f32).reshape(ntr, 8, _L)
            acc = acc + vj * p[None, :, j * _L:(j + 1) * _L]
        return acc

    def o_cols(acc, l):
        return jnp.sum(acc, axis=-1, keepdims=True) * (gbuf[...] / l)[None]

    def wo_apply(ob, r0):
        n = ob.shape[0]
        w = wobuf[pl.ds(r0, n * 8), :].astype(f32).reshape(n, 8, D)
        return [jnp.sum(w[:, :, c * _L:(c + 1) * _L] * ob, axis=0) for c in range(ncb)]

    rest = _strided(run_slots(wo_hbm, wobuf, wo_early, 14, S_WO) + run_slots(w1_hbm, w1buf, D, 12, S_W1)
                    + run_slots(w3_hbm, w3buf, D, 12, S_W3) + run_slots(w2_hbm, w2buf, F, 12, S_W2),
                    _REST_STRIDE)
    start_all(_strided(run_slots(wq_hbm, wqbuf, D, 14, S_WQ), _WQ_STRIDE)
              + [[(x_hbm, xbuf, S_X), (gw_hbm, gwbuf, S_GW)]] + rest[:_REST_AHEAD])
    wait_for(xbuf, S_X)
    wait_for(gwbuf, S_GW)
    wait_for(wqbuf, S_WQ)
    x_row = xbuf[0].astype(f32)
    x8 = jnp.broadcast_to(x_row, (8, D)).astype(bf16)
    gdot = jnp.sum(x_row * gwbuf[...].astype(f32).reshape(1, D), axis=-1, keepdims=True)
    gbuf[...] = jnp.broadcast_to(jax.nn.sigmoid(gdot), gbuf.shape)
    for hp in range(H // 2):
        q2 = jnp.dot(x8, wqbuf[:, hp * 2 * DH:(hp + 1) * 2 * DH], preferred_element_type=f32)
        qbuf[2 * hp] = q2[:, :DH]
        qbuf[2 * hp + 1] = q2[:, DH:]
    start_all(rest[_REST_AHEAD:])
    start_all(kv_jobs(k_hbm, kbuf.at[0], 0, _KV_SPLIT, lambda s: S_K))
    wait_for(wobuf.at[pl.ds(0, wo_early), :], S_WO)
    wait_for(w1buf, S_W1)
    wait_for(w3buf, S_W3)
    wait_for(w2buf, S_W2)
    gate = jnp.dot(x8, w1buf[...], preferred_element_type=f32)
    start_all(kv_jobs(v_hbm, vbuf.at[0], 0, _KV_SPLIT, lambda s: S_V))
    up = jnp.dot(x8, w3buf[...], preferred_element_type=f32)
    hbuf[...] = gate * jax.nn.sigmoid(gate) * up

    lslot = (H - 1) % 2

    def last_jobs():
        slots = kv_jobs(v_hbm, vbuf.at[lslot], H - 1, _LAST_SPLIT, lambda s: S_VL + s)
        for g, (t0, n) in enumerate(_spans(_HOLD)):
            for t in range(t0, t0 + n, 2):
                slots += [[], [rect(wo_hbm, wobuf, wo_early // 8 + t, 2, 0, ncb, S_HOLD + g)]]
        return slots

    def head_body(h, carry):
        slot = h % 2
        nslot = 1 - slot
        start_all(kv_jobs(k_hbm, kbuf.at[nslot], h + 1, _KV_SPLIT, lambda s: S_K + nslot))
        wait_for(kbuf.at[slot], S_K + slot)
        p, l = scores(h, kbuf.at[slot])

        @pl.when(h == 0)
        def _():
            b_out = jnp.dot(hbuf[...].astype(bf16), w2buf[...], preferred_element_type=f32)
            row0 = lax.broadcasted_iota(jnp.int32, (8, D), 0) == 0
            accbuf[...] = jnp.where(row0, (1.0 - gbuf[:, 0:1]) * b_out, 0.0)

        @pl.when(h < H - 2)
        def _():
            start_all(kv_jobs(v_hbm, vbuf.at[nslot], h + 1, _KV_SPLIT, lambda s: S_V + nslot))

        @pl.when(h == H - 2)
        def _():
            start_all(last_jobs()[:_LAST_AHEAD])

        wait_for(vbuf.at[slot], S_V + slot)
        acc = pv(vbuf.at[slot], jnp.zeros((ntr, 8, _L), f32), p, 0, W // _L)
        parts = wo_apply(o_cols(acc, l), pl.multiple_of(h * DH, DH))
        accbuf[...] += jnp.concatenate(parts, axis=-1)
        return carry

    lax.fori_loop(0, H - 1, head_body, 0)

    start_all(last_jobs()[_LAST_AHEAD:], first=_LAST_AHEAD)
    vb = vbuf.at[lslot]
    wait_for(kbuf.at[lslot], S_K + lslot)
    p, l = scores(H - 1, kbuf.at[lslot])
    acc = jnp.zeros((ntr, 8, _L), f32)
    for s, (c, z) in enumerate(_spans(_LAST_SPLIT)):
        wait_for(vb.at[:, pl.ds(c * _L, z * _L)], S_VL + s)
        acc = pv(vb, acc, p, c, c + z)
    ob = o_cols(acc, l)
    tot = [accbuf[:, c * _L:(c + 1) * _L] for c in range(ncb)]
    for g, (t0, n) in enumerate(_spans(_HOLD)):
        r0 = wo_early + t0 * 8
        wait_for(wobuf.at[pl.ds(r0, n * 8), :], S_HOLD + g)
        tot = [a + b for a, b in zip(tot, wo_apply(ob[t0:t0 + n], r0))]
    for c in range(ncb):
        o_ref[0, :, c * _L:(c + 1) * _L] = jnp.sum(tot[c], axis=0, keepdims=True).astype(o_ref.dtype)


def _build(B, Sq, D, H, SK, DH, F, dtype, interpret=False):
    W = min(4096, max(256, SK // 4))
    bf16 = jnp.bfloat16
    f32 = jnp.float32
    assert B == 1 and Sq == 1 and dtype == bf16 and H % 2 == 0 and H > 2
    assert sum(_KV_SPLIT) * _L == W and sum(_LAST_SPLIT) * _L == W and sum(_HOLD) * 8 == DH
    assert all(n % 2 == 0 for n in _HOLD) and (len(_LAST_SPLIT) * (DH // 8)) % 2 == 0
    assert D % _L == 0 and F % _L == 0 and (2 * DH) % _L == 0 and (SK - W) % _L == 0
    return pl.pallas_call(
        functools.partial(_kernel, H=H, DH=DH, SK=SK, W=W, D=D, F=F),
        in_specs=[pl.BlockSpec(memory_space=pl.ANY)] * 9,
        out_specs=pl.BlockSpec(memory_space=pltpu.VMEM),
        out_shape=jax.ShapeDtypeStruct((B, Sq, D), dtype),
        scratch_shapes=[
            pltpu.VMEM((1, 1, D), bf16),
            pltpu.VMEM((D,), bf16),
            pltpu.VMEM((D, H * DH), bf16),
            pltpu.VMEM((H * DH, D), bf16),
            pltpu.VMEM((D, F), bf16),
            pltpu.VMEM((D, F), bf16),
            pltpu.VMEM((F, D), bf16),
            pltpu.VMEM((2, DH, W), bf16),
            pltpu.VMEM((2, DH, W), bf16),
            pltpu.VMEM((H, 8, DH), f32),
            pltpu.VMEM((8, F), f32),
            pltpu.VMEM((8, _L), f32),
            pltpu.VMEM((8, D), f32),
            pltpu.SemaphoreType.DMA((11 + len(_LAST_SPLIT) + len(_HOLD),)),
        ],
        compiler_params=pltpu.CompilerParams(vmem_limit_bytes=64 * 1024 * 1024,
                                             disable_bounds_checks=True,
                                             disable_semaphore_checks=True),
        interpret=interpret,
    )


@jax.jit
def pallas_gated_mix__sliding_block_cached__glu_gated_swiglu__decode_kernel(
    A_x: jax.Array,
    A_k_cache: jax.Array,
    A_v_cache: jax.Array,
    A_wq: jax.Array,
    A_wo: jax.Array,
    B_x: jax.Array,
    B_w1: jax.Array,
    B_w3: jax.Array,
    B_w2: jax.Array,
    gate_w: jax.Array,
):
    B, Sq, D = A_x.shape
    _, H, SK, DH = A_k_cache.shape
    assert A_wq.shape == (D, H * DH)
    kt = jnp.swapaxes(A_k_cache, 2, 3)
    vt = jnp.swapaxes(A_v_cache, 2, 3)
    call = _build(B, Sq, D, H, SK, DH, B_w1.shape[1], A_x.dtype)
    return call(A_x, gate_w, A_wq, kt, vt, A_wo, B_w1, B_w3, B_w2)
```

```python
import functools

import jax
import jax.numpy as jnp
from jax import lax
import jax.experimental.pallas as pl
import jax.experimental.pallas.tpu as pltpu

_L = 128
_KV_SPLIT = (6, 8, 4, 4, 10)
_LAST_SPLIT = (6, 8, 8, 6, 4)
_HOLD = (18, 4, 2)
_RUN = 16
_WQ_STRIDE = 24
_REST_STRIDE = 16
_REST_AHEAD = 48
_LAST_AHEAD = 48


def _spans(split):
    out, c = [], 0
    for z in split:
        out.append((c, z))
        c += z
    return out


def _kernel(x_hbm, gw_hbm, wq_hbm, k_hbm, v_hbm, wo_hbm, w1_hbm, w3_hbm, w2_hbm,
            o_ref,
            xbuf, gwbuf, wqbuf, wobuf, w1buf, w3buf, w2buf, kbuf, vbuf,
            qbuf, hbuf, gbuf, accbuf,
            sems,
            *, H, DH, SK, W, D, F):
    f32 = jnp.float32
    bf16 = jnp.bfloat16
    scale = DH ** -0.5
    s0 = SK - W
    ntr = DH // 8
    ncb = D // _L
    S_X, S_GW, S_WQ, S_W1, S_W3, S_W2, S_WO, S_K, S_V, S_VL = 0, 1, 2, 3, 4, 5, 6, 7, 9, 11
    S_HOLD = S_VL + len(_LAST_SPLIT)
    wo_early = (H - 1) * DH

    def start_all(slots):
        for i, slot in enumerate(slots):
            for src, dst, sem in slot:
                pltpu.make_async_copy(src, dst, sems.at[sem]).start(priority=i % 2)

    def wait_for(ref, sem):
        pltpu.make_async_copy(ref, ref, sems.at[sem]).wait()

    def kv_slots(src, buf, h, split, sem_of):
        return [[(src.at[0, h, pl.ds(d * 8, 8), pl.ds(s0 + c * _L, z * _L)],
                  buf.at[pl.ds(d * 8, 8), pl.ds(c * _L, z * _L)], sem_of(s))]
                for s, (c, z) in enumerate(_spans(split)) for d in range(ntr)]

    def rect(src, dst, t, nt, c, nc, sem):
        idx = (pl.ds(t * 8, nt * 8), pl.ds(c * _L, nc * _L))
        return (src.at[idx], dst.at[idx], sem)

    def add_runs(runs, src, dst, nrows, base, sem):
        cw = src.shape[1] // _L
        nt = nrows // 8 * cw
        cuts = sorted(set([0, nt] + list(range(-base % _RUN, nt, _RUN))))
        for s, e in zip(cuts[:-1], cuts[1:]):
            slot = runs.setdefault((base + s) // _RUN, [])
            if s % cw:
                m = min(e, (s // cw + 1) * cw)
                slot.append(rect(src, dst, s // cw, 1, s % cw, m - s, sem))
                s = m
            if e - s >= cw:
                n = (e - s) // cw
                slot.append(rect(src, dst, s // cw, n, 0, cw, sem))
                s += n * cw
            if e > s:
                slot.append(rect(src, dst, s // cw, 1, 0, e - s, sem))

    def sweeps(runs, stride):
        slots = []
        for r in sorted(runs, key=lambda r: (r % stride, r)):
            if len(slots) % 2 != (r // stride) % 2:
                slots.append([])
            slots.append(runs[r])
        return slots + [[]] * (len(slots) % 2)

    def scores(h, kb):
        q = qbuf[h].astype(bf16)
        s = jnp.dot(q, kb[...], preferred_element_type=f32)
        m = jnp.max(s, axis=-1, keepdims=True)
        p = jnp.exp((s - m) * scale)
        return p, jnp.sum(p, axis=-1, keepdims=True)

    def pv(vb, acc, p, j0, j1):
        for j in range(j0, j1):
            vj = vb[:, j * _L:(j + 1) * _L].astype(f32).reshape(ntr, 8, _L)
            acc = acc + vj * p[None, :, j * _L:(j + 1) * _L]
        return acc

    def o_cols(acc, l):
        return jnp.sum(acc, axis=-1, keepdims=True) * (gbuf[...] / l)[None]

    def wo_apply(ob, r0):
        n = ob.shape[0]
        w = wobuf[pl.ds(r0, n * 8), :].astype(f32).reshape(n, 8, D)
        return [jnp.sum(w[:, :, c * _L:(c + 1) * _L] * ob, axis=0) for c in range(ncb)]

    t_wo, t_ff = H * DH * D // 1024, D * F // 1024
    wq_runs, rest_runs = {}, {}
    add_runs(wq_runs, wq_hbm, wqbuf, D, 2, S_WQ)
    add_runs(rest_runs, wo_hbm, wobuf, wo_early, 2, S_WO)
    add_runs(rest_runs, w1_hbm, w1buf, D, 4 + t_wo, S_W1)
    add_runs(rest_runs, w3_hbm, w3buf, D, 4 + t_wo + t_ff, S_W3)
    add_runs(rest_runs, w2_hbm, w2buf, F, 4 + t_wo + 2 * t_ff, S_W2)
    rest = sweeps(rest_runs, _REST_STRIDE)

    start_all(sweeps(wq_runs, _WQ_STRIDE))
    start_all([[(x_hbm, xbuf, S_X)], [(gw_hbm, gwbuf, S_GW)]])
    start_all(rest[:_REST_AHEAD])
    wait_for(xbuf, S_X)
    wait_for(gwbuf, S_GW)
    wait_for(wqbuf, S_WQ)
    x_row = xbuf[0].astype(f32)
    x8 = jnp.broadcast_to(x_row, (8, D)).astype(bf16)
    gdot = jnp.sum(x_row * gwbuf[...].astype(f32).reshape(1, D), axis=-1, keepdims=True)
    gbuf[...] = jnp.broadcast_to(jax.nn.sigmoid(gdot), gbuf.shape)
    for hp in range(H // 2):
        q2 = jnp.dot(x8, wqbuf[:, hp * 2 * DH:(hp + 1) * 2 * DH], preferred_element_type=f32)
        qbuf[2 * hp] = q2[:, :DH]
        qbuf[2 * hp + 1] = q2[:, DH:]
    start_all(rest[_REST_AHEAD:])
    start_all(kv_slots(k_hbm, kbuf.at[0], 0, _KV_SPLIT, lambda s: S_K))
    wait_for(wobuf.at[pl.ds(0, wo_early), :], S_WO)
    wait_for(w1buf, S_W1)
    wait_for(w3buf, S_W3)
    wait_for(w2buf, S_W2)
    gate = jnp.dot(x8, w1buf[...], preferred_element_type=f32)
    start_all(kv_slots(v_hbm, vbuf.at[0], 0, _KV_SPLIT, lambda s: S_V))
    up = jnp.dot(x8, w3buf[...], preferred_element_type=f32)
    hbuf[...] = gate * jax.nn.sigmoid(gate) * up

    lslot = (H - 1) % 2

    def last_slots():
        slots = kv_slots(v_hbm, vbuf.at[lslot], H - 1, _LAST_SPLIT, lambda s: S_VL + s)
        for g, (t0, n) in enumerate(_spans(_HOLD)):
            slots += [[], [rect(wo_hbm, wobuf, wo_early // 8 + t0, n, 0, ncb, S_HOLD + g)]]
        return slots

    def head_body(h, carry):
        slot = h % 2
        nslot = 1 - slot
        start_all(kv_slots(k_hbm, kbuf.at[nslot], h + 1, _KV_SPLIT, lambda s: S_K + nslot))
        wait_for(kbuf.at[slot], S_K + slot)
        p, l = scores(h, kbuf.at[slot])

        @pl.when(h == 0)
        def _():
            b_out = jnp.dot(hbuf[...].astype(bf16), w2buf[...], preferred_element_type=f32)
            row0 = lax.broadcasted_iota(jnp.int32, (8, D), 0) == 0
            accbuf[...] = jnp.where(row0, (1.0 - gbuf[:, 0:1]) * b_out, 0.0)

        @pl.when(h < H - 2)
        def _():
            start_all(kv_slots(v_hbm, vbuf.at[nslot], h + 1, _KV_SPLIT, lambda s: S_V + nslot))

        @pl.when(h == H - 2)
        def _():
            start_all(last_slots()[:_LAST_AHEAD])

        wait_for(vbuf.at[slot], S_V + slot)
        acc = pv(vbuf.at[slot], jnp.zeros((ntr, 8, _L), f32), p, 0, W // _L)
        parts = wo_apply(o_cols(acc, l), pl.multiple_of(h * DH, DH))
        accbuf[...] += jnp.concatenate(parts, axis=-1)
        return carry

    lax.fori_loop(0, H - 1, head_body, 0)

    start_all(last_slots()[_LAST_AHEAD:])
    vb = vbuf.at[lslot]
    wait_for(kbuf.at[lslot], S_K + lslot)
    p, l = scores(H - 1, kbuf.at[lslot])
    acc = jnp.zeros((ntr, 8, _L), f32)
    for s, (c, z) in enumerate(_spans(_LAST_SPLIT)):
        wait_for(vb.at[:, pl.ds(c * _L, z * _L)], S_VL + s)
        acc = pv(vb, acc, p, c, c + z)
    ob = o_cols(acc, l)
    tot = [accbuf[:, c * _L:(c + 1) * _L] for c in range(ncb)]
    for g, (t0, n) in enumerate(_spans(_HOLD)):
        r0 = wo_early + t0 * 8
        wait_for(wobuf.at[pl.ds(r0, n * 8), :], S_HOLD + g)
        tot = [a + b for a, b in zip(tot, wo_apply(ob[t0:t0 + n], r0))]
    for c in range(ncb):
        o_ref[0, :, c * _L:(c + 1) * _L] = jnp.sum(tot[c], axis=0, keepdims=True).astype(o_ref.dtype)


def _build(B, Sq, D, H, SK, DH, F, dtype, interpret=False):
    W = min(4096, max(256, SK // 4))
    bf16 = jnp.bfloat16
    f32 = jnp.float32
    assert B == 1 and Sq == 1 and dtype == bf16 and H % 2 == 0 and H > 2
    assert sum(_KV_SPLIT) * _L == W and sum(_LAST_SPLIT) * _L == W and sum(_HOLD) * 8 == DH
    assert DH % 16 == 0 and _REST_AHEAD % 2 == 0 and _LAST_AHEAD % 2 == 0
    assert D % _L == 0 and F % _L == 0 and (2 * DH) % _L == 0 and (SK - W) % _L == 0
    return pl.pallas_call(
        functools.partial(_kernel, H=H, DH=DH, SK=SK, W=W, D=D, F=F),
        in_specs=[pl.BlockSpec(memory_space=pl.ANY)] * 9,
        out_specs=pl.BlockSpec(memory_space=pltpu.VMEM),
        out_shape=jax.ShapeDtypeStruct((B, Sq, D), dtype),
        scratch_shapes=[
            pltpu.VMEM((1, 1, D), bf16),
            pltpu.VMEM((D,), bf16),
            pltpu.VMEM((D, H * DH), bf16),
            pltpu.VMEM((H * DH, D), bf16),
            pltpu.VMEM((D, F), bf16),
            pltpu.VMEM((D, F), bf16),
            pltpu.VMEM((F, D), bf16),
            pltpu.VMEM((2, DH, W), bf16),
            pltpu.VMEM((2, DH, W), bf16),
            pltpu.VMEM((H, 8, DH), f32),
            pltpu.VMEM((8, F), f32),
            pltpu.VMEM((8, _L), f32),
            pltpu.VMEM((8, D), f32),
            pltpu.SemaphoreType.DMA((11 + len(_LAST_SPLIT) + len(_HOLD),)),
        ],
        compiler_params=pltpu.CompilerParams(vmem_limit_bytes=64 * 1024 * 1024,
                                             disable_bounds_checks=True,
                                             disable_semaphore_checks=True),
        interpret=interpret,
    )


@jax.jit
def pallas_gated_mix__sliding_block_cached__glu_gated_swiglu__decode_kernel(
    A_x: jax.Array,
    A_k_cache: jax.Array,
    A_v_cache: jax.Array,
    A_wq: jax.Array,
    A_wo: jax.Array,
    B_x: jax.Array,
    B_w1: jax.Array,
    B_w3: jax.Array,
    B_w2: jax.Array,
    gate_w: jax.Array,
):
    B, Sq, D = A_x.shape
    _, H, SK, DH = A_k_cache.shape
    assert A_wq.shape == (D, H * DH)
    kt = jnp.swapaxes(A_k_cache, 2, 3)
    vt = jnp.swapaxes(A_v_cache, 2, 3)
    call = _build(B, Sq, D, H, SK, DH, B_w1.shape[1], A_x.dtype)
    return call(A_x, gate_w, A_wq, kt, vt, A_wo, B_w1, B_w3, B_w2)
```

```python
import functools

import jax
import jax.numpy as jnp
from jax import lax
import jax.experimental.pallas as pl
import jax.experimental.pallas.tpu as pltpu

_L = 128
_KV_SPLIT = (6, 8, 4, 4, 10)
_LAST_SPLIT = (6, 8, 8, 6, 4)
_HOLD = (18, 4, 2)
_RUN = 16
_WQ_STRIDE = 24
_REST_STRIDE = 48
_REST_AHEAD = 48
_LAST_AHEAD = 48


def _spans(split):
    out, c = [], 0
    for z in split:
        out.append((c, z))
        c += z
    return out


def _kernel(x_hbm, gw_hbm, wq_hbm, k_hbm, v_hbm, wo_hbm, w1_hbm, w3_hbm, w2_hbm,
            o_ref,
            xbuf, gwbuf, wqbuf, wobuf, w1buf, w3buf, w2buf, kbuf, vbuf,
            qbuf, hbuf, gbuf, accbuf,
            sems,
            *, H, DH, SK, W, D, F):
    f32 = jnp.float32
    bf16 = jnp.bfloat16
    scale = DH ** -0.5
    s0 = SK - W
    ntr = DH // 8
    ncb = D // _L
    S_X, S_GW, S_WQ, S_W1, S_W3, S_W2, S_WO, S_K, S_V, S_VL = 0, 1, 2, 3, 4, 5, 6, 7, 9, 11
    S_HOLD = S_VL + len(_LAST_SPLIT)
    wo_early = (H - 1) * DH

    def start_all(slots):
        for i, slot in enumerate(slots):
            for src, dst, sem in slot:
                pltpu.make_async_copy(src, dst, sems.at[sem]).start(priority=i % 2)

    def wait_for(ref, sem):
        pltpu.make_async_copy(ref, ref, sems.at[sem]).wait()

    def kv_slots(src, buf, h, split, sem_of):
        return [[(src.at[0, h, pl.ds(d * 8, 8), pl.ds(s0 + c * _L, z * _L)],
                  buf.at[pl.ds(d * 8, 8), pl.ds(c * _L, z * _L)], sem_of(s))]
                for s, (c, z) in enumerate(_spans(split)) for d in range(ntr)]

    def rect(src, dst, t, nt, c, nc, sem):
        idx = (pl.ds(t * 8, nt * 8), pl.ds(c * _L, nc * _L))
        return (src.at[idx], dst.at[idx], sem)

    def add_runs(runs, src, dst, nrows, base, sem):
        cw = src.shape[1] // _L
        nt = nrows // 8 * cw
        cuts = sorted(set([0, nt] + list(range(-base % _RUN, nt, _RUN))))
        for s, e in zip(cuts[:-1], cuts[1:]):
            slot = runs.setdefault((base + s) // _RUN, [])
            if s % cw:
                m = min(e, (s // cw + 1) * cw)
                slot.append(rect(src, dst, s // cw, 1, s % cw, m - s, sem))
                s = m
            if e - s >= cw:
                n = (e - s) // cw
                slot.append(rect(src, dst, s // cw, n, 0, cw, sem))
                s += n * cw
            if e > s:
                slot.append(rect(src, dst, s // cw, 1, 0, e - s, sem))

    def sweeps(runs, stride):
        slots = []
        for r in sorted(runs, key=lambda r: (r % stride, r)):
            if len(slots) % 2 != (r // stride) % 2:
                slots.append([])
            slots.append(runs[r])
        return slots + [[]] * (len(slots) % 2)

    def scores(h, kb):
        q = qbuf[h].astype(bf16)
        s = jnp.dot(q, kb[...], preferred_element_type=f32)
        m = jnp.max(s, axis=-1, keepdims=True)
        p = jnp.exp((s - m) * scale)
        return p, jnp.sum(p, axis=-1, keepdims=True)

    def pv(vb, acc, p, j0, j1):
        for j in range(j0, j1):
            vj = vb[:, j * _L:(j + 1) * _L].astype(f32).reshape(ntr, 8, _L)
            acc = acc + vj * p[None, :, j * _L:(j + 1) * _L]
        return acc

    def o_cols(acc, l):
        return jnp.sum(acc, axis=-1, keepdims=True) * (gbuf[...] / l)[None]

    def wo_apply(ob, r0):
        n = ob.shape[0]
        w = wobuf[pl.ds(r0, n * 8), :].astype(f32).reshape(n, 8, D)
        return [jnp.sum(w[:, :, c * _L:(c + 1) * _L] * ob, axis=0) for c in range(ncb)]

    t_ff = D * F // 1024
    wq_runs, rest_runs = {}, {}
    add_runs(wq_runs, wq_hbm, wqbuf, D, 2, S_WQ)
    add_runs(rest_runs, w2_hbm, w2buf, F, 0, S_W2)
    add_runs(rest_runs, w3_hbm, w3buf, D, t_ff, S_W3)
    add_runs(rest_runs, w1_hbm, w1buf, D, 2 * t_ff, S_W1)
    add_runs(rest_runs, wo_hbm, wobuf, wo_early, 3 * t_ff + 2, S_WO)
    rest = sweeps(rest_runs, _REST_STRIDE)

    start_all(sweeps(wq_runs, _WQ_STRIDE))
    start_all([[(x_hbm, xbuf, S_X)], [(gw_hbm, gwbuf, S_GW)]])
    start_all(rest[:_REST_AHEAD])
    wait_for(xbuf, S_X)
    wait_for(gwbuf, S_GW)
    wait_for(wqbuf, S_WQ)
    x_row = xbuf[0].astype(f32)
    x8 = jnp.broadcast_to(x_row, (8, D)).astype(bf16)
    gdot = jnp.sum(x_row * gwbuf[...].astype(f32).reshape(1, D), axis=-1, keepdims=True)
    gbuf[...] = jnp.broadcast_to(jax.nn.sigmoid(gdot), gbuf.shape)
    for hp in range(H // 2):
        q2 = jnp.dot(x8, wqbuf[:, hp * 2 * DH:(hp + 1) * 2 * DH], preferred_element_type=f32)
        qbuf[2 * hp] = q2[:, :DH]
        qbuf[2 * hp + 1] = q2[:, DH:]
    start_all(rest[_REST_AHEAD:])
    start_all(kv_slots(k_hbm, kbuf.at[0], 0, _KV_SPLIT, lambda s: S_K))
    wait_for(wobuf.at[pl.ds(0, wo_early), :], S_WO)
    wait_for(w1buf, S_W1)
    wait_for(w3buf, S_W3)
    wait_for(w2buf, S_W2)
    gate = jnp.dot(x8, w1buf[...], preferred_element_type=f32)
    start_all(kv_slots(v_hbm, vbuf.at[0], 0, _KV_SPLIT, lambda s: S_V))
    up = jnp.dot(x8, w3buf[...], preferred_element_type=f32)
    hbuf[...] = gate * jax.nn.sigmoid(gate) * up

    lslot = (H - 1) % 2

    def last_slots():
        slots = kv_slots(v_hbm, vbuf.at[lslot], H - 1, _LAST_SPLIT, lambda s: S_VL + s)
        for g, (t0, n) in enumerate(_spans(_HOLD)):
            slots += [[], [rect(wo_hbm, wobuf, wo_early // 8 + t0, n, 0, ncb, S_HOLD + g)]]
        return slots

    def head_body(h, carry):
        slot = h % 2
        nslot = 1 - slot
        start_all(kv_slots(k_hbm, kbuf.at[nslot], h + 1, _KV_SPLIT, lambda s: S_K + nslot))
        wait_for(kbuf.at[slot], S_K + slot)
        p, l = scores(h, kbuf.at[slot])

        @pl.when(h == 0)
        def _():
            b_out = jnp.dot(hbuf[...].astype(bf16), w2buf[...], preferred_element_type=f32)
            row0 = lax.broadcasted_iota(jnp.int32, (8, D), 0) == 0
            accbuf[...] = jnp.where(row0, (1.0 - gbuf[:, 0:1]) * b_out, 0.0)

        @pl.when(h < H - 2)
        def _():
            start_all(kv_slots(v_hbm, vbuf.at[nslot], h + 1, _KV_SPLIT, lambda s: S_V + nslot))

        @pl.when(h == H - 2)
        def _():
            start_all(last_slots()[:_LAST_AHEAD])

        wait_for(vbuf.at[slot], S_V + slot)
        acc = pv(vbuf.at[slot], jnp.zeros((ntr, 8, _L), f32), p, 0, W // _L)
        parts = wo_apply(o_cols(acc, l), pl.multiple_of(h * DH, DH))
        accbuf[...] += jnp.concatenate(parts, axis=-1)
        return carry

    lax.fori_loop(0, H - 1, head_body, 0)

    start_all(last_slots()[_LAST_AHEAD:])
    vb = vbuf.at[lslot]
    wait_for(kbuf.at[lslot], S_K + lslot)
    p, l = scores(H - 1, kbuf.at[lslot])
    acc = jnp.zeros((ntr, 8, _L), f32)
    for s, (c, z) in enumerate(_spans(_LAST_SPLIT)):
        wait_for(vb.at[:, pl.ds(c * _L, z * _L)], S_VL + s)
        acc = pv(vb, acc, p, c, c + z)
    ob = o_cols(acc, l)
    tot = [accbuf[:, c * _L:(c + 1) * _L] for c in range(ncb)]
    for g, (t0, n) in enumerate(_spans(_HOLD)):
        r0 = wo_early + t0 * 8
        wait_for(wobuf.at[pl.ds(r0, n * 8), :], S_HOLD + g)
        tot = [a + b for a, b in zip(tot, wo_apply(ob[t0:t0 + n], r0))]
    for c in range(ncb):
        o_ref[0, :, c * _L:(c + 1) * _L] = jnp.sum(tot[c], axis=0, keepdims=True).astype(o_ref.dtype)


def _build(B, Sq, D, H, SK, DH, F, dtype, interpret=False):
    W = min(4096, max(256, SK // 4))
    bf16 = jnp.bfloat16
    f32 = jnp.float32
    assert B == 1 and Sq == 1 and dtype == bf16 and H % 2 == 0 and H > 2
    assert sum(_KV_SPLIT) * _L == W and sum(_LAST_SPLIT) * _L == W and sum(_HOLD) * 8 == DH
    assert DH % 16 == 0 and _REST_AHEAD % 2 == 0 and _LAST_AHEAD % 2 == 0
    assert D % _L == 0 and F % _L == 0 and (2 * DH) % _L == 0 and (SK - W) % _L == 0
    return pl.pallas_call(
        functools.partial(_kernel, H=H, DH=DH, SK=SK, W=W, D=D, F=F),
        in_specs=[pl.BlockSpec(memory_space=pl.ANY)] * 9,
        out_specs=pl.BlockSpec(memory_space=pltpu.VMEM),
        out_shape=jax.ShapeDtypeStruct((B, Sq, D), dtype),
        scratch_shapes=[
            pltpu.VMEM((1, 1, D), bf16),
            pltpu.VMEM((D,), bf16),
            pltpu.VMEM((D, H * DH), bf16),
            pltpu.VMEM((H * DH, D), bf16),
            pltpu.VMEM((D, F), bf16),
            pltpu.VMEM((D, F), bf16),
            pltpu.VMEM((F, D), bf16),
            pltpu.VMEM((2, DH, W), bf16),
            pltpu.VMEM((2, DH, W), bf16),
            pltpu.VMEM((H, 8, DH), f32),
            pltpu.VMEM((8, F), f32),
            pltpu.VMEM((8, _L), f32),
            pltpu.VMEM((8, D), f32),
            pltpu.SemaphoreType.DMA((11 + len(_LAST_SPLIT) + len(_HOLD),)),
        ],
        compiler_params=pltpu.CompilerParams(vmem_limit_bytes=64 * 1024 * 1024,
                                             disable_bounds_checks=True,
                                             disable_semaphore_checks=True),
        interpret=interpret,
    )


@jax.jit
def pallas_gated_mix__sliding_block_cached__glu_gated_swiglu__decode_kernel(
    A_x: jax.Array,
    A_k_cache: jax.Array,
    A_v_cache: jax.Array,
    A_wq: jax.Array,
    A_wo: jax.Array,
    B_x: jax.Array,
    B_w1: jax.Array,
    B_w3: jax.Array,
    B_w2: jax.Array,
    gate_w: jax.Array,
):
    B, Sq, D = A_x.shape
    _, H, SK, DH = A_k_cache.shape
    assert A_wq.shape == (D, H * DH)
    kt = jnp.swapaxes(A_k_cache, 2, 3)
    vt = jnp.swapaxes(A_v_cache, 2, 3)
    call = _build(B, Sq, D, H, SK, DH, B_w1.shape[1], A_x.dtype)
    return call(A_x, gate_w, A_wq, kt, vt, A_wo, B_w1, B_w3, B_w2)
```

```python
import functools

import jax
import jax.numpy as jnp
from jax import lax
import jax.experimental.pallas as pl
import jax.experimental.pallas.tpu as pltpu

_L = 128
_KV_SPLIT = (6, 8, 4, 4, 10)
_LAST_SPLIT = (6, 8, 8, 6, 4)
_HOLD = (18, 4, 2)
_RUN = 16
_WQ_STRIDE = 24
_REST_STRIDE = 48
_REST_AHEAD = 48
_LAST_AHEAD = 48
_WARMUP = 20


def _spans(split):
    out, c = [], 0
    for z in split:
        out.append((c, z))
        c += z
    return out


def _kernel(x_hbm, gw_hbm, wq_hbm, k_hbm, v_hbm, wo_hbm, w1_hbm, w3_hbm, w2_hbm,
            o_ref,
            xbuf, gwbuf, wqbuf, wobuf, w1buf, w3buf, w2buf, kbuf, vbuf,
            qbuf, gbuf, accbuf,
            sems,
            *, H, DH, SK, W, D, F):
    f32 = jnp.float32
    bf16 = jnp.bfloat16
    scale = DH ** -0.5
    s0 = SK - W
    ntr = DH // 8
    ncb = D // _L
    S_X, S_GW, S_WQ, S_W1, S_W3, S_W2, S_WO, S_K, S_V, S_VL = 0, 1, 2, 3, 4, 5, 6, 7, 9, 11
    S_HOLD = S_VL + len(_LAST_SPLIT)
    wo_early = (H - 1) * DH

    def start_all(slots):
        for i, slot in enumerate(slots):
            for src, dst, sem in slot:
                pltpu.make_async_copy(src, dst, sems.at[sem]).start(priority=i % 2)

    def wait_for(ref, sem):
        pltpu.make_async_copy(ref, ref, sems.at[sem]).wait()

    def kv_slots(src, buf, h, split, sem_of):
        return [[(src.at[0, h, pl.ds(d * 8, 8), pl.ds(s0 + c * _L, z * _L)],
                  buf.at[pl.ds(d * 8, 8), pl.ds(c * _L, z * _L)], sem_of(s))]
                for s, (c, z) in enumerate(_spans(split)) for d in range(ntr)]

    def rect(src, dst, t, nt, c, nc, sem):
        idx = (pl.ds(t * 8, nt * 8), pl.ds(c * _L, nc * _L))
        return (src.at[idx], dst.at[idx], sem)

    def add_runs(runs, src, dst, nrows, base, sem):
        cw = src.shape[1] // _L
        nt = nrows // 8 * cw
        cuts = sorted(set([0, nt] + list(range(-base % _RUN, nt, _RUN))))
        for s, e in zip(cuts[:-1], cuts[1:]):
            slot = runs.setdefault((base + s) // _RUN, [])
            if s % cw:
                m = min(e, (s // cw + 1) * cw)
                slot.append(rect(src, dst, s // cw, 1, s % cw, m - s, sem))
                s = m
            if e - s >= cw:
                n = (e - s) // cw
                slot.append(rect(src, dst, s // cw, n, 0, cw, sem))
                s += n * cw
            if e > s:
                slot.append(rect(src, dst, s // cw, 1, 0, e - s, sem))

    def sweeps(runs, stride):
        slots = []
        for r in sorted(runs, key=lambda r: (r % stride, r)):
            if len(slots) % 2 != (r // stride) % 2:
                slots.append([])
            slots.append(runs[r])
        return slots + [[]] * (len(slots) % 2)

    def scores(h, kb):
        q = qbuf[h].astype(bf16)
        s = jnp.dot(q, kb[...], preferred_element_type=f32)
        m = jnp.max(s, axis=-1, keepdims=True)
        p = jnp.exp((s - m) * scale)
        return p, jnp.sum(p, axis=-1, keepdims=True)

    def pv(vb, acc, p, j0, j1):
        for j in range(j0, j1):
            vj = vb[:, j * _L:(j + 1) * _L].astype(f32).reshape(ntr, 8, _L)
            acc = acc + vj * p[None, :, j * _L:(j + 1) * _L]
        return acc

    def o_cols(acc, l):
        return jnp.sum(acc, axis=-1, keepdims=True) * (gbuf[...] / l)[None]

    def wo_apply(ob, r0):
        n = ob.shape[0]
        w = wobuf[pl.ds(r0, n * 8), :].astype(f32).reshape(n, 8, D)
        return [jnp.sum(w[:, :, c * _L:(c + 1) * _L] * ob, axis=0) for c in range(ncb)]

    t_ff = D * F // 1024
    wq_runs, rest_runs = {}, {}
    add_runs(wq_runs, wq_hbm, wqbuf, D, 2, S_WQ)
    add_runs(rest_runs, w2_hbm, w2buf, F, 0, S_W2)
    add_runs(rest_runs, w3_hbm, w3buf, D, t_ff, S_W3)
    add_runs(rest_runs, w1_hbm, w1buf, D, 2 * t_ff, S_W1)
    add_runs(rest_runs, wo_hbm, wobuf, wo_early, 3 * t_ff + 2, S_WO)
    rest = sweeps(rest_runs, _REST_STRIDE)

    k0 = kv_slots(k_hbm, kbuf.at[0], 0, _KV_SPLIT, lambda s: S_K)
    start_all([[], [job for slot in k0[:_WARMUP] for job in slot]] + k0[_WARMUP:])
    start_all(sweeps(wq_runs, _WQ_STRIDE))
    start_all([[(x_hbm, xbuf, S_X)], [(gw_hbm, gwbuf, S_GW)]])
    start_all(rest[:_REST_AHEAD])
    wait_for(xbuf, S_X)
    wait_for(gwbuf, S_GW)
    wait_for(wqbuf, S_WQ)
    x_row = xbuf[0].astype(f32)
    x8 = jnp.broadcast_to(x_row, (8, D)).astype(bf16)
    gdot = jnp.sum(x_row * gwbuf[...].astype(f32).reshape(1, D), axis=-1, keepdims=True)
    gbuf[...] = jnp.broadcast_to(jax.nn.sigmoid(gdot), gbuf.shape)
    for hp in range(H // 2):
        q2 = jnp.dot(x8, wqbuf[:, hp * 2 * DH:(hp + 1) * 2 * DH], preferred_element_type=f32)
        qbuf[2 * hp] = q2[:, :DH]
        qbuf[2 * hp + 1] = q2[:, DH:]
    start_all(rest[_REST_AHEAD:])
    start_all(kv_slots(v_hbm, vbuf.at[0], 0, _KV_SPLIT, lambda s: S_V))
    wait_for(wobuf.at[pl.ds(0, wo_early), :], S_WO)
    wait_for(w1buf, S_W1)
    wait_for(w3buf, S_W3)
    wait_for(w2buf, S_W2)
    start_all(kv_slots(k_hbm, kbuf.at[1], 1, _KV_SPLIT, lambda s: S_K + 1))
    gate = jnp.dot(x8, w1buf[...], preferred_element_type=f32)
    up = jnp.dot(x8, w3buf[...], preferred_element_type=f32)
    hid = (gate * jax.nn.sigmoid(gate) * up).astype(bf16)
    b_out = jnp.dot(hid, w2buf[...], preferred_element_type=f32)
    row0 = lax.broadcasted_iota(jnp.int32, (8, D), 0) == 0
    accbuf[...] = jnp.where(row0, (1.0 - gbuf[:, 0:1]) * b_out, 0.0)

    lslot = (H - 1) % 2

    def last_slots():
        slots = kv_slots(v_hbm, vbuf.at[lslot], H - 1, _LAST_SPLIT, lambda s: S_VL + s)
        for g, (t0, n) in enumerate(_spans(_HOLD)):
            slots += [[], [rect(wo_hbm, wobuf, wo_early // 8 + t0, n, 0, ncb, S_HOLD + g)]]
        return slots

    def head(h, slot, issue_a, issue_b):
        wait_for(kbuf.at[slot], S_K + slot)
        start_all(issue_a())
        p, l = scores(h, kbuf.at[slot])
        wait_for(vbuf.at[slot], S_V + slot)
        start_all(issue_b())
        acc = pv(vbuf.at[slot], jnp.zeros((ntr, 8, _L), f32), p, 0, W // _L)
        r0 = h * DH if isinstance(h, int) else pl.multiple_of(h * DH, DH)
        accbuf[...] += jnp.concatenate(wo_apply(o_cols(acc, l), r0), axis=-1)

    def head_body(h, carry):
        slot = h % 2
        nslot = 1 - slot
        head(h, slot,
             lambda: kv_slots(v_hbm, vbuf.at[nslot], h + 1, _KV_SPLIT, lambda s: S_V + nslot),
             lambda: kv_slots(k_hbm, kbuf.at[slot], h + 2, _KV_SPLIT, lambda s: S_K + slot))
        return carry

    lax.fori_loop(0, H - 2, head_body, 0)
    head(H - 2, (H - 2) % 2, lambda: last_slots()[:_LAST_AHEAD], lambda: last_slots()[_LAST_AHEAD:])

    vb = vbuf.at[lslot]
    wait_for(kbuf.at[lslot], S_K + lslot)
    p, l = scores(H - 1, kbuf.at[lslot])
    acc = jnp.zeros((ntr, 8, _L), f32)
    for s, (c, z) in enumerate(_spans(_LAST_SPLIT)):
        wait_for(vb.at[:, pl.ds(c * _L, z * _L)], S_VL + s)
        acc = pv(vb, acc, p, c, c + z)
    ob = o_cols(acc, l)
    tot = [accbuf[:, c * _L:(c + 1) * _L] for c in range(ncb)]
    for g, (t0, n) in enumerate(_spans(_HOLD)):
        r0 = wo_early + t0 * 8
        wait_for(wobuf.at[pl.ds(r0, n * 8), :], S_HOLD + g)
        tot = [a + b for a, b in zip(tot, wo_apply(ob[t0:t0 + n], r0))]
    for c in range(ncb):
        o_ref[0, :, c * _L:(c + 1) * _L] = jnp.sum(tot[c], axis=0, keepdims=True).astype(o_ref.dtype)


def _build(B, Sq, D, H, SK, DH, F, dtype, interpret=False):
    W = min(4096, max(256, SK // 4))
    bf16 = jnp.bfloat16
    f32 = jnp.float32
    assert B == 1 and Sq == 1 and dtype == bf16 and H % 2 == 0 and H > 2
    assert sum(_KV_SPLIT) * _L == W and sum(_LAST_SPLIT) * _L == W and sum(_HOLD) * 8 == DH
    assert DH % 16 == 0 and _REST_AHEAD % 2 == 0 and _LAST_AHEAD % 2 == 0 and _WARMUP % 2 == 0
    assert D % _L == 0 and F % _L == 0 and (2 * DH) % _L == 0 and (SK - W) % _L == 0
    return pl.pallas_call(
        functools.partial(_kernel, H=H, DH=DH, SK=SK, W=W, D=D, F=F),
        in_specs=[pl.BlockSpec(memory_space=pl.ANY)] * 9,
        out_specs=pl.BlockSpec(memory_space=pltpu.VMEM),
        out_shape=jax.ShapeDtypeStruct((B, Sq, D), dtype),
        scratch_shapes=[
            pltpu.VMEM((1, 1, D), bf16),
            pltpu.VMEM((D,), bf16),
            pltpu.VMEM((D, H * DH), bf16),
            pltpu.VMEM((H * DH, D), bf16),
            pltpu.VMEM((D, F), bf16),
            pltpu.VMEM((D, F), bf16),
            pltpu.VMEM((F, D), bf16),
            pltpu.VMEM((2, DH, W), bf16),
            pltpu.VMEM((2, DH, W), bf16),
            pltpu.VMEM((H, 8, DH), f32),
            pltpu.VMEM((8, _L), f32),
            pltpu.VMEM((8, D), f32),
            pltpu.SemaphoreType.DMA((11 + len(_LAST_SPLIT) + len(_HOLD),)),
        ],
        compiler_params=pltpu.CompilerParams(vmem_limit_bytes=64 * 1024 * 1024,
                                             disable_bounds_checks=True,
                                             disable_semaphore_checks=True),
        interpret=interpret,
    )


@jax.jit
def pallas_gated_mix__sliding_block_cached__glu_gated_swiglu__decode_kernel(
    A_x: jax.Array,
    A_k_cache: jax.Array,
    A_v_cache: jax.Array,
    A_wq: jax.Array,
    A_wo: jax.Array,
    B_x: jax.Array,
    B_w1: jax.Array,
    B_w3: jax.Array,
    B_w2: jax.Array,
    gate_w: jax.Array,
):
    B, Sq, D = A_x.shape
    _, H, SK, DH = A_k_cache.shape
    assert A_wq.shape == (D, H * DH)
    kt = jnp.swapaxes(A_k_cache, 2, 3)
    vt = jnp.swapaxes(A_v_cache, 2, 3)
    call = _build(B, Sq, D, H, SK, DH, B_w1.shape[1], A_x.dtype)
    return call(A_x, gate_w, A_wq, kt, vt, A_wo, B_w1, B_w3, B_w2)
```

```python
import functools

import jax
import jax.numpy as jnp
import numpy as np
from jax import lax
import jax.experimental.pallas as pl
import jax.experimental.pallas.tpu as pltpu

_L = 128
_KV_SPLIT = (6, 8, 4, 4, 10)
_LAST_SPLIT = (6, 8, 8, 6, 4)
_HOLD = (18, 4, 2)
_RUN = 16
_WQ_STRIDE = 24
_REST_STRIDE = 48
_REST_AHEAD = 48
_LAST_AHEAD = 48
_WARMUP = 20


def _spans(split):
    out, c = [], 0
    for z in split:
        out.append((c, z))
        c += z
    return out


def _kernel(x_hbm, gw_hbm, wq_hbm, k_hbm, v_hbm, wo_hbm, w1_hbm, w3_hbm, w2_hbm,
            o_ref,
            xbuf, gwbuf, wqbuf, wobuf, w1buf, w3buf, w2buf, kbuf, vbuf,
            qbuf, gbuf, accbuf,
            sems,
            *, H, DH, SK, W, D, F):
    f32 = jnp.float32
    bf16 = jnp.bfloat16
    scale = float(np.asarray(DH ** -0.5, dtype=bf16))
    s0 = SK - W
    ntr = DH // 8
    ncb = D // _L
    S_X, S_GW, S_WQ, S_W1, S_W3, S_W2, S_WO, S_K, S_V, S_VL = 0, 1, 2, 3, 4, 5, 6, 7, 9, 11
    S_HOLD = S_VL + len(_LAST_SPLIT)
    wo_early = (H - 1) * DH

    def start_all(slots):
        for i, slot in enumerate(slots):
            for src, dst, sem in slot:
                pltpu.make_async_copy(src, dst, sems.at[sem]).start(priority=i % 2)

    def wait_for(ref, sem):
        pltpu.make_async_copy(ref, ref, sems.at[sem]).wait()

    def kv_slots(src, buf, h, split, sem_of):
        return [[(src.at[0, h, pl.ds(d * 8, 8), pl.ds(s0 + c * _L, z * _L)],
                  buf.at[pl.ds(d * 8, 8), pl.ds(c * _L, z * _L)], sem_of(s))]
                for s, (c, z) in enumerate(_spans(split)) for d in range(ntr)]

    def rect(src, dst, t, nt, c, nc, sem):
        idx = (pl.ds(t * 8, nt * 8), pl.ds(c * _L, nc * _L))
        return (src.at[idx], dst.at[idx], sem)

    def add_runs(runs, src, dst, nrows, base, sem):
        cw = src.shape[1] // _L
        nt = nrows // 8 * cw
        cuts = sorted(set([0, nt] + list(range(-base % _RUN, nt, _RUN))))
        for s, e in zip(cuts[:-1], cuts[1:]):
            slot = runs.setdefault((base + s) // _RUN, [])
            if s % cw:
                m = min(e, (s // cw + 1) * cw)
                slot.append(rect(src, dst, s // cw, 1, s % cw, m - s, sem))
                s = m
            if e - s >= cw:
                n = (e - s) // cw
                slot.append(rect(src, dst, s // cw, n, 0, cw, sem))
                s += n * cw
            if e > s:
                slot.append(rect(src, dst, s // cw, 1, 0, e - s, sem))

    def sweeps(runs, stride):
        slots = []
        for r in sorted(runs, key=lambda r: (r % stride, r)):
            if len(slots) % 2 != (r // stride) % 2:
                slots.append([])
            slots.append(runs[r])
        return slots + [[]] * (len(slots) % 2)

    def scores(h, kb):
        q = qbuf[h].astype(bf16)
        s = jnp.dot(q, kb[...], preferred_element_type=f32)
        s = (s.astype(bf16).astype(f32) * scale).astype(bf16).astype(f32)
        p = jnp.exp(s - jnp.max(s, axis=-1, keepdims=True))
        return p, jnp.sum(p, axis=-1, keepdims=True)

    def pv(vb, acc, p, j0, j1):
        for j in range(j0, j1):
            vj = vb[:, j * _L:(j + 1) * _L].astype(f32).reshape(ntr, 8, _L)
            acc = acc + vj * p[None, :, j * _L:(j + 1) * _L]
        return acc

    def o_cols(acc, l):
        return jnp.sum(acc, axis=-1, keepdims=True) * (gbuf[...] / l)[None]

    def wo_apply(ob, r0):
        n = ob.shape[0]
        w = wobuf[pl.ds(r0, n * 8), :].astype(f32).reshape(n, 8, D)
        return [jnp.sum(w[:, :, c * _L:(c + 1) * _L] * ob, axis=0) for c in range(ncb)]

    t_ff = D * F // 1024
    wq_runs, rest_runs = {}, {}
    add_runs(wq_runs, wq_hbm, wqbuf, D, 2, S_WQ)
    add_runs(rest_runs, w2_hbm, w2buf, F, 0, S_W2)
    add_runs(rest_runs, w3_hbm, w3buf, D, t_ff, S_W3)
    add_runs(rest_runs, w1_hbm, w1buf, D, 2 * t_ff, S_W1)
    add_runs(rest_runs, wo_hbm, wobuf, wo_early, 3 * t_ff + 2, S_WO)
    rest = sweeps(rest_runs, _REST_STRIDE)

    k0 = kv_slots(k_hbm, kbuf.at[0], 0, _KV_SPLIT, lambda s: S_K)
    start_all([[], [job for slot in k0[:_WARMUP] for job in slot]] + k0[_WARMUP:])
    start_all(sweeps(wq_runs, _WQ_STRIDE))
    start_all([[(x_hbm, xbuf, S_X)], [(gw_hbm, gwbuf, S_GW)]])
    start_all(rest[:_REST_AHEAD])
    wait_for(xbuf, S_X)
    wait_for(gwbuf, S_GW)
    wait_for(wqbuf, S_WQ)
    x_row = xbuf[0].astype(f32)
    x8 = jnp.broadcast_to(x_row, (8, D)).astype(bf16)
    gdot = jnp.sum(x_row * gwbuf[...].astype(f32).reshape(1, D), axis=-1, keepdims=True)
    gbuf[...] = jnp.broadcast_to(jax.nn.sigmoid(gdot), gbuf.shape)
    for hp in range(H // 2):
        q2 = jnp.dot(x8, wqbuf[:, hp * 2 * DH:(hp + 1) * 2 * DH], preferred_element_type=f32)
        qbuf[2 * hp] = q2[:, :DH]
        qbuf[2 * hp + 1] = q2[:, DH:]
    start_all(rest[_REST_AHEAD:])
    start_all(kv_slots(v_hbm, vbuf.at[0], 0, _KV_SPLIT, lambda s: S_V))
    wait_for(wobuf.at[pl.ds(0, wo_early), :], S_WO)
    wait_for(w1buf, S_W1)
    wait_for(w3buf, S_W3)
    wait_for(w2buf, S_W2)
    start_all(kv_slots(k_hbm, kbuf.at[1], 1, _KV_SPLIT, lambda s: S_K + 1))
    gate = jnp.dot(x8, w1buf[...], preferred_element_type=f32)
    up = jnp.dot(x8, w3buf[...], preferred_element_type=f32)
    hid = (gate * jax.nn.sigmoid(gate) * up).astype(bf16)
    b_out = jnp.dot(hid, w2buf[...], preferred_element_type=f32)
    row0 = lax.broadcasted_iota(jnp.int32, (8, D), 0) == 0
    accbuf[...] = jnp.where(row0, (1.0 - gbuf[:, 0:1]) * b_out, 0.0)

    lslot = (H - 1) % 2

    def last_slots():
        slots = kv_slots(v_hbm, vbuf.at[lslot], H - 1, _LAST_SPLIT, lambda s: S_VL + s)
        for g, (t0, n) in enumerate(_spans(_HOLD)):
            slots += [[], [rect(wo_hbm, wobuf, wo_early // 8 + t0, n, 0, ncb, S_HOLD + g)]]
        return slots

    def head(h, slot, issue_a, issue_b):
        wait_for(kbuf.at[slot], S_K + slot)
        start_all(issue_a())
        p, l = scores(h, kbuf.at[slot])
        wait_for(vbuf.at[slot], S_V + slot)
        start_all(issue_b())
        acc = pv(vbuf.at[slot], jnp.zeros((ntr, 8, _L), f32), p, 0, W // _L)
        r0 = h * DH if isinstance(h, int) else pl.multiple_of(h * DH, DH)
        accbuf[...] += jnp.concatenate(wo_apply(o_cols(acc, l), r0), axis=-1)

    def head_body(h, carry):
        slot = h % 2
        nslot = 1 - slot
        head(h, slot,
             lambda: kv_slots(v_hbm, vbuf.at[nslot], h + 1, _KV_SPLIT, lambda s: S_V + nslot),
             lambda: kv_slots(k_hbm, kbuf.at[slot], h + 2, _KV_SPLIT, lambda s: S_K + slot))
        return carry

    lax.fori_loop(0, H - 2, head_body, 0)
    head(H - 2, (H - 2) % 2, lambda: last_slots()[:_LAST_AHEAD], lambda: last_slots()[_LAST_AHEAD:])

    vb = vbuf.at[lslot]
    wait_for(kbuf.at[lslot], S_K + lslot)
    p, l = scores(H - 1, kbuf.at[lslot])
    acc = jnp.zeros((ntr, 8, _L), f32)
    for s, (c, z) in enumerate(_spans(_LAST_SPLIT)):
        wait_for(vb.at[:, pl.ds(c * _L, z * _L)], S_VL + s)
        acc = pv(vb, acc, p, c, c + z)
    ob = o_cols(acc, l)
    tot = [accbuf[:, c * _L:(c + 1) * _L] for c in range(ncb)]
    for g, (t0, n) in enumerate(_spans(_HOLD)):
        r0 = wo_early + t0 * 8
        wait_for(wobuf.at[pl.ds(r0, n * 8), :], S_HOLD + g)
        tot = [a + b for a, b in zip(tot, wo_apply(ob[t0:t0 + n], r0))]
    for c in range(ncb):
        o_ref[0, :, c * _L:(c + 1) * _L] = jnp.sum(tot[c], axis=0, keepdims=True).astype(o_ref.dtype)


def _build(B, Sq, D, H, SK, DH, F, dtype, interpret=False):
    W = min(4096, max(256, SK // 4))
    bf16 = jnp.bfloat16
    f32 = jnp.float32
    assert B == 1 and Sq == 1 and dtype == bf16 and H % 2 == 0 and H > 2
    assert sum(_KV_SPLIT) * _L == W and sum(_LAST_SPLIT) * _L == W and sum(_HOLD) * 8 == DH
    assert DH % 16 == 0 and _REST_AHEAD % 2 == 0 and _LAST_AHEAD % 2 == 0 and _WARMUP % 2 == 0
    assert D % _L == 0 and F % _L == 0 and (2 * DH) % _L == 0 and (SK - W) % _L == 0
    return pl.pallas_call(
        functools.partial(_kernel, H=H, DH=DH, SK=SK, W=W, D=D, F=F),
        in_specs=[pl.BlockSpec(memory_space=pl.ANY)] * 9,
        out_specs=pl.BlockSpec(memory_space=pltpu.VMEM),
        out_shape=jax.ShapeDtypeStruct((B, Sq, D), dtype),
        scratch_shapes=[
            pltpu.VMEM((1, 1, D), bf16),
            pltpu.VMEM((D,), bf16),
            pltpu.VMEM((D, H * DH), bf16),
            pltpu.VMEM((H * DH, D), bf16),
            pltpu.VMEM((D, F), bf16),
            pltpu.VMEM((D, F), bf16),
            pltpu.VMEM((F, D), bf16),
            pltpu.VMEM((2, DH, W), bf16),
            pltpu.VMEM((2, DH, W), bf16),
            pltpu.VMEM((H, 8, DH), f32),
            pltpu.VMEM((8, _L), f32),
            pltpu.VMEM((8, D), f32),
            pltpu.SemaphoreType.DMA((11 + len(_LAST_SPLIT) + len(_HOLD),)),
        ],
        compiler_params=pltpu.CompilerParams(vmem_limit_bytes=64 * 1024 * 1024,
                                             disable_bounds_checks=True,
                                             disable_semaphore_checks=True),
        interpret=interpret,
    )


@jax.jit
def pallas_gated_mix__sliding_block_cached__glu_gated_swiglu__decode_kernel(
    A_x: jax.Array,
    A_k_cache: jax.Array,
    A_v_cache: jax.Array,
    A_wq: jax.Array,
    A_wo: jax.Array,
    B_x: jax.Array,
    B_w1: jax.Array,
    B_w3: jax.Array,
    B_w2: jax.Array,
    gate_w: jax.Array,
):
    B, Sq, D = A_x.shape
    _, H, SK, DH = A_k_cache.shape
    assert A_wq.shape == (D, H * DH)
    kt = jnp.swapaxes(A_k_cache, 2, 3)
    vt = jnp.swapaxes(A_v_cache, 2, 3)
    call = _build(B, Sq, D, H, SK, DH, B_w1.shape[1], A_x.dtype)
    return call(A_x, gate_w, A_wq, kt, vt, A_wo, B_w1, B_w3, B_w2)
```
